```python
import jax
import jax.numpy as jnp

def _softmax(x, axis=-1):
    return jax.nn.softmax(x, axis=axis)

def _gelu(x):
    return jax.nn.gelu(x, approximate=True)

def _silu(x):
    return jax.nn.silu(x)

def _sigmoid(x):
    return jax.nn.sigmoid(x)

def _layernorm(x, axis=-1, eps=1e-05):
    m = jnp.mean(x, axis=axis, keepdims=True)
    v = jnp.var(x, axis=axis, keepdims=True)
    return (x - m) / jnp.sqrt(v + eps)

def _scatter_add(tgt, idx, src, axis=0):
    return tgt.at[idx].add(src)

def _segment_sum(src, seg, n):
    return jax.ops.segment_sum(src, seg, n)

class _Rng:

    def __init__(self, key):
        self._k = key

    def _next(self):
        self._k, sub = jax.random.split(self._k)
        return sub

    def normal(self, shape):
        return jax.random.normal(self._next(), shape, dtype=jnp.bfloat16)

    def randint(self, lo, hi, shape):
        return jax.random.randint(self._next(), shape, lo, hi, dtype=jnp.int32)

    def uniform(self, shape, lo=0.0, hi=1.0):
        return jax.random.uniform(self._next(), shape, jnp.bfloat16, lo, hi)

    def permutation(self, n):
        return jax.random.permutation(self._next(), n)
kernel_name = 'sequential_preLN__ssm_conv_s4__mixer_gmlp__prompt'

def _fwd_setup_inputs():
    _rng = _Rng(jax.random.key(int.from_bytes(__import__("os").urandom(4), "little")))
    _w = lambda a: (lambda t: t.astype(jnp.bfloat16) if jnp.issubdtype(t.dtype, jnp.floating) else t)(jnp.asarray(a))

    def _A_setup():
        B, L, D, N = (1, 2048, 576, 128)
        A_re = -jnp.exp((lambda *s: _rng.normal(s) * 0.05)(D, N))
        A_im = jnp.pi * (lambda *s: _rng.normal(s) * 0.05)(D, N)
        B_re = (lambda *s: _rng.normal(s) * 0.05)(D, N)
        B_im = (lambda *s: _rng.normal(s) * 0.05)(D, N)
        C_re = (lambda *s: _rng.normal(s) * 0.05)(D, N)
        C_im = (lambda *s: _rng.normal(s) * 0.05)(D, N)
        log_dt = (lambda *s: _rng.normal(s) * 0.05)(D) * 0.5 - 4.0
        Dskip = (lambda *s: _rng.normal(s) * 0.05)(D)
        return {'u': _w((lambda *s: _rng.normal(s) * 0.05)(B, L, D)), 'A_re': _w(A_re), 'A_im': _w(A_im), 'B_re': _w(B_re), 'B_im': _w(B_im), 'C_re': _w(C_re), 'C_im': _w(C_im), 'log_dt': _w(log_dt), 'Dskip': _w(Dskip)}
    _A_in = _A_setup()

    def _B_setup():
        B, S, D, F = (1, 2048, 576, 4608)
        Fh = F // 2
        return {'x': _w((lambda *s: _rng.normal(s) * 0.05)(B, S, D)), 'w_in': _w((lambda *s: _rng.normal(s) * 0.05)(D, 2 * Fh)), 'w_sp': _w(0.01 * (lambda *s: _rng.normal(s) * 0.05)(S, S)), 'b_sp': _w(1.0 + 0.01 * (lambda *s: _rng.normal(s) * 0.05)(S)), 'w_out': _w((lambda *s: _rng.normal(s) * 0.05)(Fh, D))}
    _B_in = _B_setup()
    return {'A_u': _A_in['u'], 'A_A_re': _A_in['A_re'], 'A_A_im': _A_in['A_im'], 'A_B_re': _A_in['B_re'], 'A_B_im': _A_in['B_im'], 'A_C_re': _A_in['C_re'], 'A_C_im': _A_in['C_im'], 'A_log_dt': _A_in['log_dt'], 'A_Dskip': _A_in['Dskip'], 'B_x': _B_in['x'], 'B_w_in': _B_in['w_in'], 'B_w_sp': _B_in['w_sp'], 'B_b_sp': _B_in['b_sp'], 'B_w_out': _B_in['w_out']}

def _fwd_reference(A_u, A_A_re, A_A_im, A_B_re, A_B_im, A_C_re, A_C_im, A_log_dt, A_Dskip, B_x, B_w_in, B_w_sp, B_b_sp, B_w_out):

    def _A_ref(u, A_re, A_im, B_re, B_im, C_re, C_im, log_dt, Dskip):
        Bsz, L, D = u.shape
        dt = jnp.exp(log_dt)[:, None]
        A = A_re + 1j * A_im
        Bc = B_re + 1j * B_im
        Cc = C_re + 1j * C_im
        logdA = dt * A
        dB = dt * Bc
        l = (lambda x, dt: x.astype(dt))(jnp.arange(L), A_re.dtype)
        P = jnp.exp(logdA[:, :, None] * l[None, None, :])
        K = jnp.einsum('dn,dnl,dn->dl', Cc, P, dB).real
        L2 = 2 * L
        Kp = jnp.pad(K, ((0, 0), (0, L)))
        up = (lambda x, *d: x.transpose(*d))(u, 0, 2, 1)
        up = jnp.pad(up, ((0, 0), (0, 0), (0, L)))
        Kf = (lambda x, axes=(-2, -1): jnp.fft.rfft2(x.astype(jnp.float32), axes=axes))(Kp[:, None, :], axes=(-2, -1))
        Uf = (lambda x, axes=(-2, -1): jnp.fft.rfft2(x.astype(jnp.float32), axes=axes))(up[:, :, None, :], axes=(-2, -1))
        Yf = Uf * Kf[None, :, :, :]
        y = (lambda x, s, axes=(-2, -1): jnp.fft.irfft2(x, s=s, axes=axes).astype(jnp.bfloat16))(Yf, (1, L2), axes=(-2, -1))[:, :, 0, :L]
        y = (lambda x, *d: x.transpose(*d))(y, 0, 2, 1) + u * Dskip[None, None, :]
        return y

    def _B_ref(x, w_in, w_sp, b_sp, w_out):
        B, S, D = x.shape
        F = w_in.shape[-1]
        Fh = F // 2
        z = _gelu(jnp.einsum('bsd,df->bsf', x, w_in))
        z1 = z[..., :Fh].copy()
        z2 = _layernorm(z[..., Fh:], axis=-1)
        g = jnp.einsum('ts,bsf->btf', w_sp, z2) + b_sp[None, :, None]
        return jnp.einsum('bsf,fd->bsd', z1 * g, w_out)
    x = A_u
    h = x + _A_ref(_layernorm(x, axis=-1), A_A_re, A_A_im, A_B_re, A_B_im, A_C_re, A_C_im, A_log_dt, A_Dskip)
    h2 = h + _B_ref(_layernorm(h, axis=-1), B_w_in, B_w_sp, B_b_sp, B_w_out)
    return h2

def setup_inputs():
    _inp = _fwd_setup_inputs()
    _gk = jax.random.fold_in(jax.random.key(int.from_bytes(__import__("os").urandom(4), "little")), 2 ** 31 - 1)
    _shapes = [[1, 2048, 576]]
    _dtypes = ['bfloat16']
    _gks = jax.random.split(_gk, len(_shapes))
    _gs = [jax.random.normal(k, s, dtype=jnp.dtype(d)) * 0.05 for k, s, d in zip(_gks, _shapes, _dtypes)]
    _inp['grad_out'] = _gs[0]
    return _inp

def reference(A_u, A_A_re, A_A_im, A_B_re, A_B_im, A_C_re, A_C_im, A_log_dt, A_Dskip, B_w_in, B_w_sp, B_b_sp, B_w_out, B_x, grad_out):
    _const = dict(B_x=B_x)

    def _f(*_d):
        return _fwd_reference(**{'A_u': _d[0], 'A_A_re': _d[1], 'A_A_im': _d[2], 'A_B_re': _d[3], 'A_B_im': _d[4], 'A_C_re': _d[5], 'A_C_im': _d[6], 'A_log_dt': _d[7], 'A_Dskip': _d[8], 'B_w_in': _d[9], 'B_w_sp': _d[10], 'B_b_sp': _d[11], 'B_w_out': _d[12], **_const})
    _out, _vjp = jax.vjp(_f, A_u, A_A_re, A_A_im, A_B_re, A_B_im, A_C_re, A_C_im, A_log_dt, A_Dskip, B_w_in, B_w_sp, B_b_sp, B_w_out)
    _grads = _vjp(grad_out)
    _out0 = jnp.asarray(_out)
    return (_out0, *[jnp.asarray(_g) for _g in _grads])
```

```python
import numpy as np
import ml_dtypes
import jax
import jax.numpy as jnp
from jax import lax
import jax.experimental.pallas as pl
import jax.experimental.pallas.tpu as pltpu

L = 2048
D = 576
N = 128
FH = 2304
F = 2 * FH
P = 256
NB = L // P
M2 = 2 * P
EPS = 1e-5
TR = 256
F32 = jnp.float32
BF16 = jnp.bfloat16

_BLK = [(1, 256, 0), (2, 136, 1), (4, 72, 2), (4, 72, 2)] + [(8, 40, 3)] * 4


def _split(a):
    a = np.asarray(a, np.float64)
    hi = a.astype(np.float32).astype(ml_dtypes.bfloat16)
    lo = (a - hi.astype(np.float64)).astype(np.float32).astype(ml_dtypes.bfloat16)
    return hi, lo


def _consts():
    k = np.arange(P)
    om = np.pi * (2 * k + 1) / M2
    j = np.arange(P)
    fw = np.concatenate([np.cos(np.outer(om, j)), -np.sin(np.outer(om, j))], 0)
    t = np.arange(M2)
    fi = np.concatenate([np.cos(np.outer(t, om)), -np.sin(np.outer(t, om))], 1) * (2.0 / M2)
    lb = np.arange(L).astype(np.float32).astype(ml_dtypes.bfloat16).astype(np.float64).astype(np.int64)
    gs = []
    for blk in (0, 1, 2, 4):
        step = _BLK[blk][0]
        g = np.zeros((M2, P))
        for jj in range(P):
            m = (lb[blk * P + jj] - blk * P) // step
            g[:, m] += fw[:, jj]
        gs.append(g)
    gs = np.stack(gs)
    gts = np.transpose(gs, (0, 2, 1))
    out = []
    for a in (gs, gts, fi, fi.T):
        out.extend(_split(a))
    return out


def _dot(a, b):
    return jnp.dot(a, b, preferred_element_type=F32)


def _dot_nt(a, b):
    return lax.dot_general(a, b, (((1,), (1,)), ((), ())), preferred_element_type=F32)


def _dot_tn(a, b):
    return lax.dot_general(a, b, (((0,), (0,)), ((), ())), preferred_element_type=F32)


def _dot3(mh, ml, x):
    xh = x.astype(BF16)
    xl = (x - xh.astype(F32)).astype(BF16)
    return _dot(mh, xh) + (_dot(mh, xl) + _dot(ml, xh))


def _ln(x):
    mu = jnp.mean(x, axis=-1, keepdims=True)
    xc = x - mu
    var = jnp.mean(xc * xc, axis=-1, keepdims=True)
    r = lax.rsqrt(var + EPS)
    return xc * r, r


def _ln_bwd(dn, n, r):
    return r * (dn - jnp.mean(dn, axis=-1, keepdims=True)
                - n * jnp.mean(dn * n, axis=-1, keepdims=True))


_GK = 0.7978845608028654
_GC = 0.044715


def _gelu_parts(a):
    t = jnp.tanh(_GK * (a + _GC * a * a * a))
    g = 0.5 * a * (1.0 + t)
    dg = 0.5 * (1.0 + t) + 0.5 * a * (1.0 - t * t) * _GK * (1.0 + 3.0 * _GC * a * a)
    return g, dg


def _cmul(ar, ai, br, bi):
    return ar * br - ai * bi, ar * bi + ai * br


def _cexp(zr, zi, mult):
    e = jnp.exp(zr * mult)
    ang = zi * mult
    return e * jnp.cos(ang), e * jnp.sin(ang)


def _tables(zr, zi):
    i32 = lax.broadcasted_iota(jnp.int32, (32, 1), 0)
    mult = ((i32 % 8) * (1 << (i32 // 8))).astype(F32)
    br, bi = _cexp(zr, zi, mult)
    i8 = lax.broadcasted_iota(jnp.int32, (8, 1), 0)
    er, ei = _cexp(zr, zi, (8 << i8).astype(F32))
    e = lambda j: (er[j - 3:j - 2], ei[j - 3:j - 2])
    tabs = []
    for q in range(4):
        tr, ti = br[8 * q:8 * q + 8], bi[8 * q:8 * q + 8]
        b0r, b0i = tr, ti
        for j in range(3 + q, 8):
            xr, xi = _cmul(tr, ti, *e(j))
            tr = jnp.concatenate([tr, xr], 0)
            ti = jnp.concatenate([ti, xi], 0)
        if q > 0:
            xr, xi = _cmul(b0r, b0i, *e(8))
            tr = jnp.concatenate([tr, xr], 0)
            ti = jnp.concatenate([ti, xi], 0)
        tabs.append((tr, ti))
    e8, e9, e10 = e(8), e(9), e(10)
    e98 = _cmul(*e9, *e8)
    offs = [None, e8, e9, e98, e10, _cmul(*e10, *e8), _cmul(*e10, *e9), _cmul(*e10, *e98)]
    return tabs, offs


def _kernel(x_ref, ar_ref, ai_ref, br_ref, bi_ref, cr_ref, ci_ref, ldt_ref, dsk_ref,
            win_ref, wsp_ref, bsp_ref, wout_ref, go_ref,
            gh_ref, gl_ref, gth_ref, gtl_ref, fih_ref, fil_ref, fith_ref, fitl_ref,
            o_ref, dx_ref, dar_ref, dai_ref, dbr_ref, dbi_ref, dcr_ref, dci_ref,
            dldt_ref, ddsk_ref, dwin_ref, dwsp_ref, dbsp_ref, dwout_ref,
            kt_ref, v_ref, h_ref, rh_ref, prm_ref, gr_ref):
    dt = jnp.exp(ldt_ref[...].astype(F32)).astype(BF16).astype(F32)
    dsk = dsk_ref[...].astype(F32)

    kt_ref[...] = jnp.zeros(kt_ref.shape, F32)
    for idx, r in enumerate((ar_ref, ai_ref, br_ref, bi_ref, cr_ref, ci_ref)):
        prm_ref[idx] = r[...].astype(F32)

    def coef(n):
        row = lambda idx: prm_ref[idx, pl.ds(n, 1), :]
        zr, zi = dt * row(0), dt * row(1)
        dbr, dbi = dt * row(2), dt * row(3)
        cr, ci = _cmul(row(4), row(5), dbr, dbi)
        return zr, zi, cr, ci

    def kgen(n, carry):
        zr, zi, cr, ci = coef(n)
        tabs, offs = _tables(zr, zi)
        for b in range(NB):
            _, rows, q = _BLK[b]
            xr, xi = (cr, ci) if b == 0 else _cmul(cr, ci, *offs[b])
            tr, ti = tabs[q]
            kt_ref[b, 0:rows, :] += xr * tr - xi * ti
        return carry
    lax.fori_loop(0, N, kgen, 0)

    def spectra(uh_ref, kh_ref):
        for b in range(NB):
            u, _ = _ln(x_ref[b * P:(b + 1) * P, :].astype(F32))
            uh_ref[b] = _dot3(gh_ref[0], gl_ref[0], u)
            q = _BLK[b][2]
            kh_ref[b] = _dot3(gh_ref[q], gl_ref[q], kt_ref[b])

    def s4_fwd(uh_ref, kh_ref):
        spectra(uh_ref, kh_ref)
        prev = None
        for b in range(NB):
            zr = jnp.zeros((P, D), F32)
            zi = jnp.zeros((P, D), F32)
            for a in range(b + 1):
                pr, pi = _cmul(uh_ref[a, 0:P], uh_ref[a, P:M2], kh_ref[b - a, 0:P], kh_ref[b - a, P:M2])
                zr, zi = zr + pr, zi + pi
            zf = _dot3(fih_ref[...], fil_ref[...], jnp.concatenate([zr, zi], 0))
            y = zf[0:P] if prev is None else zf[0:P] + prev
            prev = zf[P:M2]
            xb = x_ref[b * P:(b + 1) * P, :].astype(F32)
            u, _ = _ln(xb)
            h = xb + y + u * dsk
            h_ref[b * P:(b + 1) * P, :] = h
            v, r = _ln(h)
            v_ref[b * P:(b + 1) * P, :] = v.astype(BF16)
            rh_ref[b * P:(b + 1) * P, :] = r

    pl.run_scoped(s4_fwd, pltpu.VMEM((NB, M2, D), F32), pltpu.VMEM((NB, M2, D), F32))

    def gmlp(a_ref, z2_ref, r2_ref, dg_ref, acc_ref):
        nt = L // TR

        def ph_c(i, c):
            rs = pl.ds(pl.multiple_of(i * TR, TR), TR)
            a = _dot(v_ref[rs, :], win_ref[...]).astype(BF16)
            a_ref[rs, :] = a
            z2, _ = _gelu_parts(a[:, FH:].astype(F32))
            n2, r2 = _ln(z2)
            z2_ref[rs, :] = n2.astype(BF16)
            r2_ref[rs, :] = r2
            return c
        lax.fori_loop(0, nt, ph_c, 0)

        acc_ref[...] = jnp.zeros(acc_ref.shape, F32)

        def ph_d(i, c):
            rs = pl.ds(pl.multiple_of(i * TR, TR), TR)
            g = _dot(wsp_ref[rs, :], z2_ref[...]) + bsp_ref[rs, :].astype(F32)
            z1, dg1 = _gelu_parts(a_ref[rs, 0:FH].astype(F32))
            m = (z1 * g).astype(BF16)
            o_ref[rs, :] = (h_ref[rs, :] + _dot(m, wout_ref[...])).astype(BF16)
            go = go_ref[rs, :]
            dm = _dot_nt(go, wout_ref[...])
            acc_ref[...] += _dot_tn(m, go)
            dg = dm * z1
            dbsp_ref[rs, :] = jnp.sum(dg, axis=-1, keepdims=True).astype(BF16)
            dgb = dg.astype(BF16)
            dg_ref[rs, :] = dgb
            dwsp_ref[rs, :] = _dot_nt(dgb, z2_ref[...]).astype(BF16)
            a_ref[rs, 0:FH] = (dm * g * dg1).astype(BF16)
            return c
        lax.fori_loop(0, nt, ph_d, 0)
        dwout_ref[...] = acc_ref[...].astype(BF16)

        def ph_e(i, c):
            rs = pl.ds(pl.multiple_of(i * TR, TR), TR)
            dn2 = _dot_tn(wsp_ref[:, rs], dg_ref[...])
            dz2 = _ln_bwd(dn2, z2_ref[rs, :].astype(F32), r2_ref[rs, :])
            _, dg2 = _gelu_parts(a_ref[rs, FH:F].astype(F32))
            a_ref[rs, FH:F] = (dz2 * dg2).astype(BF16)
            dv = _dot_nt(a_ref[rs, :], win_ref[...])
            dh = go_ref[rs, :].astype(F32) + _ln_bwd(dv, v_ref[rs, :].astype(F32), rh_ref[rs, :])
            h_ref[rs, :] = dh
            return c
        lax.fori_loop(0, nt, ph_e, 0)

        for cb in range(F // 512):
            dwin_ref[:, cb * 512:(cb + 1) * 512] = _dot_tn(
                v_ref[...], a_ref[:, cb * 512:(cb + 1) * 512]).astype(BF16)

    pl.run_scoped(gmlp, pltpu.VMEM((L, F), BF16), pltpu.VMEM((L, FH), BF16),
                  pltpu.VMEM((L, 1), F32), pltpu.VMEM((L, FH), BF16),
                  pltpu.VMEM((FH, D), F32))

    def s4_bwd(uh_ref, kh_ref, dz_ref):
        spectra(uh_ref, kh_ref)
        for b in range(NB):
            dzb = _dot3(fith_ref[:, 0:P], fitl_ref[:, 0:P], h_ref[b * P:(b + 1) * P, :])
            if b + 1 < NB:
                dzb = dzb + _dot3(fith_ref[:, P:M2], fitl_ref[:, P:M2],
                                  h_ref[(b + 1) * P:(b + 2) * P, :])
            dz_ref[b] = dzb
        ddsk = jnp.zeros((1, D), F32)
        for a in range(NB):
            sr = jnp.zeros((P, D), F32)
            si = jnp.zeros((P, D), F32)
            qr = jnp.zeros((P, D), F32)
            qi = jnp.zeros((P, D), F32)
            for dlt in range(NB - a):
                zr, zi = dz_ref[a + dlt, 0:P], dz_ref[a + dlt, P:M2]
                pr, pi = _cmul(kh_ref[dlt, 0:P], -kh_ref[dlt, P:M2], zr, zi)
                sr, si = sr + pr, si + pi
                pr, pi = _cmul(uh_ref[dlt, 0:P], -uh_ref[dlt, P:M2], zr, zi)
                qr, qi = qr + pr, qi + pi
            du = _dot3(gth_ref[0], gtl_ref[0], jnp.concatenate([sr, si], 0))
            q = _BLK[a][2]
            kt_ref[a] = _dot3(gth_ref[q], gtl_ref[q], jnp.concatenate([qr, qi], 0))
            dh = h_ref[a * P:(a + 1) * P, :]
            u, r = _ln(x_ref[a * P:(a + 1) * P, :].astype(F32))
            ddsk = ddsk + jnp.sum(dh * u, axis=0, keepdims=True)
            dx_ref[a * P:(a + 1) * P, :] = (dh + _ln_bwd(du + dh * dsk, u, r)).astype(BF16)
        ddsk_ref[...] = ddsk.astype(BF16)

    pl.run_scoped(s4_bwd, pltpu.VMEM((NB, M2, D), F32), pltpu.VMEM((NB, M2, D), F32),
                  pltpu.VMEM((NB, M2, D), F32))

    def kbwd(n, gdt):
        zr, zi, cr, ci = coef(n)
        tabs, offs = _tables(zr, zi)
        s0r = jnp.zeros((1, D), F32)
        s0i, s1r, s1i = s0r, s0r, s0r
        for b in range(NB):
            step, rows, q = _BLK[b]
            tr, ti = tabs[q]
            dk = kt_ref[b, 0:rows, :]
            m = lax.broadcasted_iota(jnp.int32, (rows, 1), 0).astype(F32) * float(step)
            dkm = dk * m
            a0r = jnp.sum(dk * tr, axis=0, keepdims=True)
            a0i = jnp.sum(dk * ti, axis=0, keepdims=True)
            a1r = jnp.sum(dkm * tr, axis=0, keepdims=True) + float(b * P) * a0r
            a1i = jnp.sum(dkm * ti, axis=0, keepdims=True) + float(b * P) * a0i
            if b > 0:
                a0r, a0i = _cmul(a0r, a0i, *offs[b])
                a1r, a1i = _cmul(a1r, a1i, *offs[b])
            s0r, s0i, s1r, s1i = s0r + a0r, s0i + a0i, s1r + a1r, s1i + a1i
        gcr, gci = s0r, -s0i
        wr, wi = _cmul(cr, ci, s1r, s1i)
        gzr, gzi = wr, -wi
        row = lambda idx: prm_ref[idx, pl.ds(n, 1), :]
        cre, cim, bre, bim = row(4), row(5), row(2), row(3)
        dbr, dbi = dt * bre, dt * bim
        gdbr = gcr * cre + gci * cim
        gdbi = gci * cre - gcr * cim
        gr_ref[4, pl.ds(n, 1), :] = gcr * dbr + gci * dbi
        gr_ref[5, pl.ds(n, 1), :] = gci * dbr - gcr * dbi
        gr_ref[2, pl.ds(n, 1), :] = dt * gdbr
        gr_ref[3, pl.ds(n, 1), :] = dt * gdbi
        gr_ref[0, pl.ds(n, 1), :] = dt * gzr
        gr_ref[1, pl.ds(n, 1), :] = dt * gzi
        return gdt + gdbr * bre + gdbi * bim + gzr * row(0) + gzi * row(1)
    gdt = lax.fori_loop(0, N, kbwd, jnp.zeros((1, D), F32))
    dldt_ref[...] = (gdt * dt).astype(BF16)
    for idx, r in enumerate((dar_ref, dai_ref, dbr_ref, dbi_ref, dcr_ref, dci_ref)):
        r[...] = gr_ref[idx].astype(BF16)


@jax.jit
def pallas_sequential_preLN__ssm_conv_s4__mixer_gmlp__prompt_kernel(
    A_u, A_A_re, A_A_im, A_B_re, A_B_im, A_C_re, A_C_im, A_log_dt, A_Dskip,
    B_x, B_w_in, B_w_sp, B_b_sp, B_w_out, grad_out,
):
    del B_x
    consts = _consts()
    sds = jax.ShapeDtypeStruct
    out_shape = (
        sds((L, D), BF16), sds((L, D), BF16),
        sds((N, D), BF16), sds((N, D), BF16), sds((N, D), BF16),
        sds((N, D), BF16), sds((N, D), BF16), sds((N, D), BF16),
        sds((1, D), BF16), sds((1, D), BF16),
        sds((D, F), BF16), sds((L, L), BF16), sds((L, 1), BF16), sds((FH, D), BF16),
    )
    outs = pl.pallas_call(
        _kernel,
        out_shape=out_shape,
        scratch_shapes=[
            pltpu.VMEM((NB, P, D), F32),
            pltpu.VMEM((L, D), BF16),
            pltpu.VMEM((L, D), F32),
            pltpu.VMEM((L, 1), F32),
            pltpu.VMEM((6, N, D), F32),
            pltpu.VMEM((6, N, D), F32),
        ],
        compiler_params=pltpu.CompilerParams(vmem_limit_bytes=120 * 1024 * 1024),
    )(A_u.reshape(L, D), A_A_re.T, A_A_im.T, A_B_re.T, A_B_im.T, A_C_re.T, A_C_im.T,
      A_log_dt.reshape(1, D), A_Dskip.reshape(1, D), B_w_in, B_w_sp,
      B_b_sp.reshape(L, 1), B_w_out, grad_out.reshape(L, D), *consts)
    (o, dx, dar, dai, dbr, dbi, dcr, dci, dldt, ddsk, dwin, dwsp, dbsp, dwout) = outs
    return (o.reshape(1, L, D), dx.reshape(1, L, D), dar.T, dai.T, dbr.T, dbi.T, dcr.T, dci.T,
            dldt.reshape(D), ddsk.reshape(D), dwin, dwsp, dbsp.reshape(L), dwout)
```

```python
import functools
import numpy as np
import ml_dtypes
import jax
import jax.numpy as jnp
from jax import lax
import jax.experimental.pallas as pl
import jax.experimental.pallas.tpu as pltpu

L = 2048
D = 576
N = 128
FH = 2304
F = 2 * FH
P = 256
NB = L // P
M2 = 2 * P
EPS = 1e-5
TR = 256
F32 = jnp.float32
BF16 = jnp.bfloat16

_BLK = [(1, 8, 32, 0), (2, 8, 16, 1), (4, 8, 8, 2), (4, 8, 8, 2)] + [(8, 4, 8, 3)] * 4
EDGE = 248
EACC = 240


def _split(a):
    a = np.asarray(a, np.float64)
    hi = a.astype(np.float32).astype(ml_dtypes.bfloat16)
    lo = (a - hi.astype(np.float64)).astype(np.float32).astype(ml_dtypes.bfloat16)
    return hi, lo


def _consts():
    k = np.arange(P)
    om = np.pi * (2 * k + 1) / M2
    j = np.arange(P)
    fw = np.concatenate([np.cos(np.outer(om, j)), -np.sin(np.outer(om, j))], 0)
    t = np.arange(M2)
    fi = np.concatenate([np.cos(np.outer(t, om)), -np.sin(np.outer(t, om))], 1) * (2.0 / M2)
    lb = np.arange(L).astype(np.float32).astype(ml_dtypes.bfloat16).astype(np.float64).astype(np.int64)
    gs = []
    for blk in (0, 1, 2, 4):
        step, nr, na, _ = _BLK[blk]
        g = np.zeros((M2, P))
        for jj in range(P):
            m = (lb[blk * P + jj] - blk * P) // step
            col = EDGE if m == nr * na else (m % nr) * na + m // nr
            g[:, col] += fw[:, jj]
        gs.append(g)
    gs.append(fw)
    gs = np.stack(gs)
    gts = np.transpose(gs, (0, 2, 1))
    out = []
    for a in (gs, gts, fi, fi.T):
        out.extend(_split(a))
    return out


def _dot(a, b):
    return jnp.dot(a, b, preferred_element_type=F32)


def _dot_nt(a, b):
    return lax.dot_general(a, b, (((1,), (1,)), ((), ())), preferred_element_type=F32)


def _dot_tn(a, b):
    return lax.dot_general(a, b, (((0,), (0,)), ((), ())), preferred_element_type=F32)


def _dot3(mh, ml, x):
    xh = x.astype(BF16)
    xl = (x - xh.astype(F32)).astype(BF16)
    return _dot(mh, xh) + (_dot(mh, xl) + _dot(ml, xh))


def _ln(x):
    mu = jnp.mean(x, axis=-1, keepdims=True)
    xc = x - mu
    var = jnp.mean(xc * xc, axis=-1, keepdims=True)
    r = lax.rsqrt(var + EPS)
    return xc * r, r


def _ln_bwd(dn, n, r):
    return r * (dn - jnp.mean(dn, axis=-1, keepdims=True)
                - n * jnp.mean(dn * n, axis=-1, keepdims=True))


_GK = 0.7978845608028654
_GC = 0.044715


def _gelu_parts(a):
    t = jnp.tanh(_GK * (a + _GC * a * a * a))
    g = 0.5 * a * (1.0 + t)
    dg = 0.5 * (1.0 + t) + 0.5 * a * (1.0 - t * t) * _GK * (1.0 + 3.0 * _GC * a * a)
    return g, dg


def _cmul(ar, ai, br, bi):
    return ar * br - ai * bi, ar * bi + ai * br


def _cexp(zr, zi, mult):
    e = jnp.exp(zr * mult)
    ang = zi * mult
    return e * jnp.cos(ang), e * jnp.sin(ang)


def _pre(pw_ref, n):
    rows = [(pw_ref[0, j, pl.ds(n, 1), :], pw_ref[1, j, pl.ds(n, 1), :]) for j in range(11)]
    e = lambda j: rows[j]
    i8 = lax.broadcasted_iota(jnp.int32, (8, 1), 0)

    def tile3(q):
        fs = []
        for bit in range(3):
            on = ((i8 >> bit) & 1) == 1
            fs.append((jnp.where(on, rows[q + bit][0], 1.0), jnp.where(on, rows[q + bit][1], 0.0)))
        return _cmul(*_cmul(*fs[0], *fs[1]), *fs[2])

    fine = [tile3(q) for q in range(4)]
    t3, t4, t5 = tile3(3), tile3(4), tile3(5)
    e6, e7, e8, e9, e10 = (e(j) for j in range(6, 11))
    e98 = _cmul(*e9, *e8)
    offs = [None, e8, e9, e98, e10, _cmul(*e10, *e8), _cmul(*e10, *e9), _cmul(*e10, *e98)]
    coarse = [[t3, _cmul(*t3, *e6), _cmul(*t3, *e7), _cmul(*t3, *_cmul(*e6, *e7))],
              [_cmul(*t4, *e8), _cmul(*t4, *_cmul(*e7, *e8))]]
    coarse += [[_cmul(*t5, *offs[b])] for b in range(2, 8)]
    edge = _cmul(*tile3(8), *e8)
    return coarse, fine, edge


def _kernel(xt_ref, ar_ref, ai_ref, br_ref, bi_ref, cr_ref, ci_ref, ldt_ref, dsk_ref,
            win_hbm, wsp_hbm, bsp_ref, woutt_ref, got_ref,
            gh_ref, gl_ref, gth_ref, gtl_ref, fih_ref, fil_ref, fith_ref, fitl_ref,
            ot_ref, dxt_ref, dar_ref, dai_ref, dbr_ref, dbi_ref, dcr_ref, dci_ref,
            dldt_ref, ddsk_ref, dwin_hbm, dwsp_hbm, dbsp_ref, dwoutt_ref,
            kt_ref, v_ref, h_ref, rh_ref, prm_ref, gr_ref, win_ref, wsp_ref, in_sem, x_ref, go_ref):
    cp_win = pltpu.make_async_copy(win_hbm, win_ref, in_sem.at[0])
    cp_wsp = pltpu.make_async_copy(wsp_hbm, wsp_ref, in_sem.at[1])
    cp_win.start()
    cp_wsp.start()
    dt = jnp.exp(ldt_ref[...].astype(F32)).astype(BF16).astype(F32)
    dsk = dsk_ref[...].astype(F32)
    for b in range(NB):
        x_ref[b * P:(b + 1) * P, :] = xt_ref[:, b * P:(b + 1) * P].astype(F32).T.astype(BF16)
        go_ref[b * P:(b + 1) * P, :] = got_ref[:, b * P:(b + 1) * P].astype(F32).T.astype(BF16)

    kt_ref[...] = jnp.zeros(kt_ref.shape, F32)
    for idx, r in enumerate((ar_ref, ai_ref, br_ref, bi_ref, cr_ref, ci_ref)):
        prm_ref[idx] = r[...].astype(F32).T

    def coef(n):
        row = lambda idx: prm_ref[idx, pl.ds(n, 1), :]
        zr, zi = dt * row(0), dt * row(1)
        dbr, dbi = dt * row(2), dt * row(3)
        cr, ci = _cmul(row(4), row(5), dbr, dbi)
        return zr, zi, cr, ci

    def powers(pw_ref):
        zr, zi = dt * prm_ref[0], dt * prm_ref[1]
        for j0 in (0, 5):
            pr, pi = _cexp(zr, zi, float(1 << j0))
            for j in range(j0, 5 if j0 == 0 else 11):
                pw_ref[0, j] = pr
                pw_ref[1, j] = pi
                pr, pi = pr * pr - pi * pi, 2.0 * pr * pi

    def kgen(pw_ref, n, carry):
        _, _, cr, ci = coef(n)
        coarse, fine, edge = _pre(pw_ref, n)
        kt_ref[1, EACC:EACC + 8, :] += cr * edge[0] - ci * edge[1]
        for q in range(4):
            ys = [(b, t, _cmul(cr, ci, *y)) for b in range(NB) if _BLK[b][3] == q
                  for t, y in enumerate(coarse[b])]
            for r in range(_BLK[ys[0][0]][1]):
                fr = jnp.broadcast_to(fine[q][0][r:r + 1], (8, D))
                fi = jnp.broadcast_to(fine[q][1][r:r + 1], (8, D))
                for b, t, (yr, yi) in ys:
                    r0 = r * _BLK[b][2] + t * 8
                    kt_ref[b, r0:r0 + 8, :] += yr * fr - yi * fi
        return carry

    def ssm_fwd(pw_ref):
        powers(pw_ref)
        lax.fori_loop(0, N, functools.partial(kgen, pw_ref), 0)
        for b in range(1, NB):
            kt_ref[b, EDGE:EDGE + 1, :] = kt_ref[1, EACC + b:EACC + b + 1, :]
        kt_ref[1, EACC:EACC + 8, :] = jnp.zeros((8, D), F32)

    with jax.named_scope('kgen'):
        pl.run_scoped(ssm_fwd, pltpu.VMEM((2, 11, N, D), F32))

    def spectra(uh_ref, kh_ref):
        for b in range(NB):
            u, _ = _ln(x_ref[b * P:(b + 1) * P, :].astype(F32))
            uh_ref[b] = _dot3(gh_ref[4], gl_ref[4], u)
            q = _BLK[b][3]
            kh_ref[b] = _dot3(gh_ref[q], gl_ref[q], kt_ref[b])

    def s4_fwd(uh_ref, kh_ref):
        spectra(uh_ref, kh_ref)
        prev = None
        for b in range(NB):
            zr = jnp.zeros((P, D), F32)
            zi = jnp.zeros((P, D), F32)
            for a in range(b + 1):
                pr, pi = _cmul(uh_ref[a, 0:P], uh_ref[a, P:M2], kh_ref[b - a, 0:P], kh_ref[b - a, P:M2])
                zr, zi = zr + pr, zi + pi
            zf = _dot3(fih_ref[...], fil_ref[...], jnp.concatenate([zr, zi], 0))
            y = zf[0:P] if prev is None else zf[0:P] + prev
            prev = zf[P:M2]
            xb = x_ref[b * P:(b + 1) * P, :].astype(F32)
            u, _ = _ln(xb)
            h = xb + y + u * dsk
            h_ref[b * P:(b + 1) * P, :] = h
            v, r = _ln(h)
            v_ref[b * P:(b + 1) * P, :] = v.astype(BF16)
            rh_ref[b * P:(b + 1) * P, :] = r

    with jax.named_scope('s4_fwd'):
        pl.run_scoped(s4_fwd, pltpu.VMEM((NB, M2, D), F32), pltpu.VMEM((NB, M2, D), F32))

    def gmlp(a_ref, z2_ref, r2_ref, dg_ref, acc_ref, sp_st, in_st, st_sem):
        nt = L // TR
        cp_win.wait()
        cp_wsp.wait()

        def sp_copy(i):
            return pltpu.make_async_copy(
                sp_st.at[i % 2], dwsp_hbm.at[pl.ds(pl.multiple_of(i * TR, TR), TR), :], st_sem.at[i % 2])

        def in_copy(cb):
            return pltpu.make_async_copy(
                in_st.at[cb % 2], dwin_hbm.at[:, cb * 512:(cb + 1) * 512], st_sem.at[2 + cb % 2])

        def ph_c(i, c):
            rs = pl.ds(pl.multiple_of(i * TR, TR), TR)
            a = _dot(v_ref[rs, :], win_ref[...]).astype(BF16)
            a_ref[rs, :] = a
            z2, _ = _gelu_parts(a[:, FH:].astype(F32))
            n2, r2 = _ln(z2)
            z2_ref[rs, :] = n2.astype(BF16)
            r2_ref[rs, :] = r2
            return c
        with jax.named_scope('ph_c'):
            lax.fori_loop(0, nt, ph_c, 0)

        acc_ref[...] = jnp.zeros(acc_ref.shape, F32)

        def ph_d(i, c):
            rs = pl.ds(pl.multiple_of(i * TR, TR), TR)
            g = _dot(wsp_ref[rs, :], z2_ref[...]) + bsp_ref[rs, :].astype(F32)
            z1, dg1 = _gelu_parts(a_ref[rs, 0:FH].astype(F32))
            m = (z1 * g).astype(BF16)
            ot_ref[:, rs] = (h_ref[rs, :] + _dot_nt(m, woutt_ref[...])).T.astype(BF16)
            dm = _dot(go_ref[rs, :], woutt_ref[...])
            acc_ref[...] += _dot(got_ref[:, rs], m)
            dg = dm * z1
            dbsp_ref[rs, :] = jnp.sum(dg, axis=-1, keepdims=True).astype(BF16)
            dgb = dg.astype(BF16)
            dg_ref[rs, :] = dgb

            @pl.when(i >= 2)
            def _():
                sp_copy(i - 2).wait()
            sp_st[i % 2] = _dot_nt(dgb, z2_ref[...]).astype(BF16)
            sp_copy(i).start()
            a_ref[rs, 0:FH] = (dm * g * dg1).astype(BF16)
            return c
        with jax.named_scope('ph_d'):
            lax.fori_loop(0, nt, ph_d, 0)
        dwoutt_ref[...] = acc_ref[...].astype(BF16)
        sp_copy(nt - 2).wait()
        sp_copy(nt - 1).wait()

        def ph_e(i, c):
            rs = pl.ds(pl.multiple_of(i * TR, TR), TR)
            dn2 = _dot_tn(wsp_ref[:, rs], dg_ref[...])
            dz2 = _ln_bwd(dn2, z2_ref[rs, :].astype(F32), r2_ref[rs, :])
            _, dg2 = _gelu_parts(a_ref[rs, FH:F].astype(F32))
            a_ref[rs, FH:F] = (dz2 * dg2).astype(BF16)
            dv = _dot_nt(a_ref[rs, :], win_ref[...])
            dh = go_ref[rs, :].astype(F32) + _ln_bwd(dv, v_ref[rs, :].astype(F32), rh_ref[rs, :])
            h_ref[rs, :] = dh
            return c
        with jax.named_scope('ph_e'):
            lax.fori_loop(0, nt, ph_e, 0)

        ncb = F // 512
        for cb in range(ncb):
            if cb >= 2:
                in_copy(cb - 2).wait()
            in_st[cb % 2] = _dot_tn(v_ref[...], a_ref[:, cb * 512:(cb + 1) * 512]).astype(BF16)
            in_copy(cb).start()
        in_copy(ncb - 2).wait()
        in_copy(ncb - 1).wait()

    pl.run_scoped(gmlp, pltpu.VMEM((L, F), BF16), pltpu.VMEM((L, FH), BF16),
                  pltpu.VMEM((L, 1), F32), pltpu.VMEM((L, FH), BF16),
                  pltpu.VMEM((D, FH), F32), pltpu.VMEM((2, TR, L), BF16),
                  pltpu.VMEM((2, D, 512), BF16), pltpu.SemaphoreType.DMA((4,)))

    def s4_bwd(uh_ref, kh_ref, dz_ref):
        spectra(uh_ref, kh_ref)
        for b in range(NB):
            dzb = _dot3(fith_ref[:, 0:P], fitl_ref[:, 0:P], h_ref[b * P:(b + 1) * P, :])
            if b + 1 < NB:
                dzb = dzb + _dot3(fith_ref[:, P:M2], fitl_ref[:, P:M2],
                                  h_ref[(b + 1) * P:(b + 2) * P, :])
            dz_ref[b] = dzb
        ddsk = jnp.zeros((1, D), F32)
        for a in range(NB):
            sr = jnp.zeros((P, D), F32)
            si = jnp.zeros((P, D), F32)
            qr = jnp.zeros((P, D), F32)
            qi = jnp.zeros((P, D), F32)
            for dlt in range(NB - a):
                zr, zi = dz_ref[a + dlt, 0:P], dz_ref[a + dlt, P:M2]
                pr, pi = _cmul(kh_ref[dlt, 0:P], -kh_ref[dlt, P:M2], zr, zi)
                sr, si = sr + pr, si + pi
                pr, pi = _cmul(uh_ref[dlt, 0:P], -uh_ref[dlt, P:M2], zr, zi)
                qr, qi = qr + pr, qi + pi
            du = _dot3(gth_ref[4], gtl_ref[4], jnp.concatenate([sr, si], 0))
            q = _BLK[a][3]
            kt_ref[a] = _dot3(gth_ref[q], gtl_ref[q], jnp.concatenate([qr, qi], 0))
            dh = h_ref[a * P:(a + 1) * P, :]
            u, r = _ln(x_ref[a * P:(a + 1) * P, :].astype(F32))
            ddsk = ddsk + jnp.sum(dh * u, axis=0, keepdims=True)
            dxt_ref[:, a * P:(a + 1) * P] = (dh + _ln_bwd(du + dh * dsk, u, r)).T.astype(BF16)
        ddsk_ref[...] = ddsk.astype(BF16)

    with jax.named_scope('s4_bwd'):
        pl.run_scoped(s4_bwd, pltpu.VMEM((NB, M2, D), F32), pltpu.VMEM((NB, M2, D), F32),
                      pltpu.VMEM((NB, M2, D), F32))

    def ssm_bwd(kv_ref, pw_ref):
        powers(pw_ref)
        kt_ref[1, EACC:EACC + 1, :] = jnp.zeros((1, D), F32)
        for b in range(1, NB):
            kt_ref[1, EACC + b:EACC + b + 1, :] = kt_ref[b, EDGE:EDGE + 1, :]
        i8 = lax.broadcasted_iota(jnp.int32, (8, 1), 0)
        kv_ref[1, EACC:EACC + 8, :] = kt_ref[1, EACC:EACC + 8, :] * ((i8 + 1) * P).astype(F32)
        for b in range(NB):
            step, nr, na, _ = _BLK[b]
            rows = nr * na
            va = (lax.broadcasted_iota(jnp.int32, (rows, 1), 0) % na) * (nr * step) + b * P
            kv_ref[b, 0:rows, :] = kt_ref[b, 0:rows, :] * va.astype(F32)

        def kbwd(n, gdt):
            _, _, cr, ci = coef(n)
            coarse, fine, edge = _pre(pw_ref, n)
            dk, dv = kt_ref[1, EACC:EACC + 8, :], kv_ref[1, EACC:EACC + 8, :]
            a0r, a0i, a1r, a1i = dk * edge[0], dk * edge[1], dv * edge[0], dv * edge[1]
            for q in range(4):
                ys = [(b, t, y) for b in range(NB) if _BLK[b][3] == q for t, y in enumerate(coarse[b])]
                for r in range(_BLK[ys[0][0]][1]):
                    w0r = w0i = w1r = w1i = None
                    for b, t, (yr, yi) in ys:
                        r0 = r * _BLK[b][2] + t * 8
                        dk, dv = kt_ref[b, r0:r0 + 8, :], kv_ref[b, r0:r0 + 8, :]
                        if w0r is None:
                            w0r, w0i, w1r, w1i = dk * yr, dk * yi, dv * yr, dv * yi
                        else:
                            w0r, w0i = w0r + dk * yr, w0i + dk * yi
                            w1r, w1i = w1r + dv * yr, w1i + dv * yi
                    vb = float(r << q)
                    w1r, w1i = w1r + vb * w0r, w1i + vb * w0i
                    fr = jnp.broadcast_to(fine[q][0][r:r + 1], (8, D))
                    fi = jnp.broadcast_to(fine[q][1][r:r + 1], (8, D))
                    pr, pi = _cmul(w0r, w0i, fr, fi)
                    a0r, a0i = a0r + pr, a0i + pi
                    pr, pi = _cmul(w1r, w1i, fr, fi)
                    a1r, a1i = a1r + pr, a1i + pi
            red = lambda t: jnp.sum(t, axis=0, keepdims=True)
            s0r, s0i, s1r, s1i = red(a0r), red(a0i), red(a1r), red(a1i)
            gcr, gci = s0r, -s0i
            wr, wi = _cmul(cr, ci, s1r, s1i)
            gzr, gzi = wr, -wi
            row = lambda idx: prm_ref[idx, pl.ds(n, 1), :]
            cre, cim, bre, bim = row(4), row(5), row(2), row(3)
            dbr, dbi = dt * bre, dt * bim
            gdbr = gcr * cre + gci * cim
            gdbi = gci * cre - gcr * cim
            gr_ref[4, pl.ds(n, 1), :] = gcr * dbr + gci * dbi
            gr_ref[5, pl.ds(n, 1), :] = gci * dbr - gcr * dbi
            gr_ref[2, pl.ds(n, 1), :] = dt * gdbr
            gr_ref[3, pl.ds(n, 1), :] = dt * gdbi
            gr_ref[0, pl.ds(n, 1), :] = dt * gzr
            gr_ref[1, pl.ds(n, 1), :] = dt * gzi
            return gdt + gdbr * bre + gdbi * bim + gzr * row(0) + gzi * row(1)
        with jax.named_scope('kbwd'):
            gdt = lax.fori_loop(0, N, kbwd, jnp.zeros((1, D), F32))
        dldt_ref[...] = (gdt * dt).astype(BF16)

    pl.run_scoped(ssm_bwd, pltpu.VMEM((NB, P, D), F32), pltpu.VMEM((2, 11, N, D), F32))
    for idx, r in enumerate((dar_ref, dai_ref, dbr_ref, dbi_ref, dcr_ref, dci_ref)):
        r[...] = gr_ref[idx].T.astype(BF16)


@jax.jit
def pallas_sequential_preLN__ssm_conv_s4__mixer_gmlp__prompt_kernel(
    A_u, A_A_re, A_A_im, A_B_re, A_B_im, A_C_re, A_C_im, A_log_dt, A_Dskip,
    B_x, B_w_in, B_w_sp, B_b_sp, B_w_out, grad_out,
):
    del B_x
    consts = _consts()
    sds = jax.ShapeDtypeStruct
    out_shape = (
        sds((D, L), BF16), sds((D, L), BF16),
        sds((D, N), BF16), sds((D, N), BF16), sds((D, N), BF16),
        sds((D, N), BF16), sds((D, N), BF16), sds((D, N), BF16),
        sds((1, D), BF16), sds((1, D), BF16),
        sds((D, F), BF16), sds((L, L), BF16), sds((L, 1), BF16), sds((D, FH), BF16),
    )
    vm = pl.BlockSpec(memory_space=pltpu.VMEM)
    hbm = pl.BlockSpec(memory_space=pl.ANY)
    outs = pl.pallas_call(
        _kernel,
        out_shape=out_shape,
        in_specs=[hbm if i in (9, 10) else vm for i in range(14 + len(consts))],
        out_specs=tuple(hbm if i in (10, 11) else vm for i in range(14)),
        scratch_shapes=[
            pltpu.VMEM((NB, P, D), F32),
            pltpu.VMEM((L, D), BF16),
            pltpu.VMEM((L, D), F32),
            pltpu.VMEM((L, 1), F32),
            pltpu.VMEM((6, N, D), F32),
            pltpu.VMEM((6, N, D), F32),
            pltpu.VMEM((D, F), BF16),
            pltpu.VMEM((L, L), BF16),
            pltpu.SemaphoreType.DMA((2,)),
            pltpu.VMEM((L, D), BF16),
            pltpu.VMEM((L, D), BF16),
        ],
        compiler_params=pltpu.CompilerParams(vmem_limit_bytes=120 * 1024 * 1024),
    )(A_u.reshape(L, D).T, A_A_re, A_A_im, A_B_re, A_B_im, A_C_re, A_C_im,
      A_log_dt.reshape(1, D), A_Dskip.reshape(1, D), B_w_in, B_w_sp,
      B_b_sp.reshape(L, 1), B_w_out.T, grad_out.reshape(L, D).T, *consts)
    (o, dx, dar, dai, dbr, dbi, dcr, dci, dldt, ddsk, dwin, dwsp, dbsp, dwout) = outs
    return (o.T.reshape(1, L, D), dx.T.reshape(1, L, D), dar, dai, dbr, dbi, dcr, dci,
            dldt.reshape(D), ddsk.reshape(D), dwin, dwsp, dbsp.reshape(L), dwout.T)
```

```python
import functools
import numpy as np
import ml_dtypes
import jax
import jax.numpy as jnp
from jax import lax
import jax.experimental.pallas as pl
import jax.experimental.pallas.tpu as pltpu

L = 2048
D = 576
N = 128
FH = 2304
F = 2 * FH
P = 128
NB = L // P
M2 = 2 * P
EPS = 1e-5
TR = 256
F32 = jnp.float32
BF16 = jnp.bfloat16

_BLK = [(1, 8, 16, 0)] * 2 + [(2, 8, 8, 1)] * 2 + [(4, 4, 8, 2)] * 4 + [(8, 2, 8, 3)] * 8
EDGE = 120
EACC = 96
ESL = 2


def _split(a):
    a = np.asarray(a, np.float64)
    hi = a.astype(np.float32).astype(ml_dtypes.bfloat16)
    lo = (a - hi.astype(np.float64)).astype(np.float32).astype(ml_dtypes.bfloat16)
    return hi, lo


def _consts():
    k = np.arange(P)
    om = np.pi * (2 * k + 1) / M2
    j = np.arange(P)
    fw = np.concatenate([np.cos(np.outer(om, j)), -np.sin(np.outer(om, j))], 0)
    t = np.arange(M2)
    fi = np.concatenate([np.cos(np.outer(t, om)), -np.sin(np.outer(t, om))], 1) * (2.0 / M2)
    lb = np.arange(L).astype(np.float32).astype(ml_dtypes.bfloat16).astype(np.float64).astype(np.int64)
    gs = []
    for blk in (0, 2, 4, 8):
        step, nr, na, _ = _BLK[blk]
        g = np.zeros((M2, P))
        for jj in range(P):
            m = (lb[blk * P + jj] - blk * P) // step
            col = EDGE if m == nr * na else (m % nr) * na + m // nr
            g[:, col] += fw[:, jj]
        gs.append(g)
    gs.append(fw)
    gs = np.stack(gs)
    gts = np.transpose(gs, (0, 2, 1))
    out = []
    for a in (gs, gts, fi, fi.T):
        out.extend(_split(a))
    return out


def _dot(a, b):
    return jnp.dot(a, b, preferred_element_type=F32)


def _dot_nt(a, b):
    return lax.dot_general(a, b, (((1,), (1,)), ((), ())), preferred_element_type=F32)


def _dot_tn(a, b):
    return lax.dot_general(a, b, (((0,), (0,)), ((), ())), preferred_element_type=F32)


def _dot3(mh, ml, x):
    xh = x.astype(BF16)
    xl = (x - xh.astype(F32)).astype(BF16)
    return _dot(mh, xh) + (_dot(mh, xl) + _dot(ml, xh))


def _dot2(mh, ml, x):
    xh = x.astype(BF16)
    return _dot(mh, xh) + _dot(ml, xh)


def _ln(x):
    mu = jnp.mean(x, axis=-1, keepdims=True)
    xc = x - mu
    var = jnp.mean(xc * xc, axis=-1, keepdims=True)
    r = lax.rsqrt(var + EPS)
    return xc * r, r


def _ln_bwd(dn, n, r):
    return r * (dn - jnp.mean(dn, axis=-1, keepdims=True)
                - n * jnp.mean(dn * n, axis=-1, keepdims=True))


_GK = 0.7978845608028654
_GC = 0.044715


def _gelu_parts(a):
    t = jnp.tanh(_GK * (a + _GC * a * a * a))
    g = 0.5 * a * (1.0 + t)
    dg = 0.5 * (1.0 + t) + 0.5 * a * (1.0 - t * t) * _GK * (1.0 + 3.0 * _GC * a * a)
    return g, dg


def _cmul(ar, ai, br, bi):
    return ar * br - ai * bi, ar * bi + ai * br


def _cexp(zr, zi, mult):
    e = jnp.exp(zr * mult)
    ang = zi * mult
    return e * jnp.cos(ang), e * jnp.sin(ang)


def _pre(pw_ref, n):
    rows = [(pw_ref[0, j, pl.ds(n, 1), :], pw_ref[1, j, pl.ds(n, 1), :]) for j in range(11)]
    e = lambda j: rows[j]
    i8 = lax.broadcasted_iota(jnp.int32, (8, 1), 0)

    def tile3(q):
        fs = []
        for bit in range(3):
            on = ((i8 >> bit) & 1) == 1
            fs.append((jnp.where(on, rows[q + bit][0], 1.0), jnp.where(on, rows[q + bit][1], 0.0)))
        return _cmul(*_cmul(*fs[0], *fs[1]), *fs[2])

    fine = [tile3(q) for q in range(4)]
    t3, t4 = tile3(3), tile3(4)
    olo = tile3(7)
    ohi = _cmul(*olo, *e(10))
    off = lambda b: tuple(x[b % 8:b % 8 + 1] for x in (olo if b < 8 else ohi))
    t36 = _cmul(*t3, *e(6))
    coarse = [[t3, t36], [_cmul(*t3, *e(7)), _cmul(*t36, *e(7))]]
    coarse += [[_cmul(*t4, *off(b))] for b in range(2, NB)]
    edge = [_cmul(*olo, *e(7)), _cmul(*ohi, *e(7))]
    return coarse, fine, edge


def _kernel(xt_hbm, ar_ref, ai_ref, br_ref, bi_ref, cr_ref, ci_ref, ldt_ref, dsk_ref,
            win_hbm, wsp_hbm, bsp_ref, woutt_hbm, got_hbm,
            c0, c1, c2, c3, c4, c5, c6, c7,
            ot_hbm, dxt_hbm, dar_ref, dai_ref, dbr_ref, dbi_ref, dcr_ref, dci_ref,
            dldt_ref, ddsk_ref, dwin_hbm, dwsp_hbm, dbsp_ref, dwoutt_hbm,
            kt_ref, v_ref, h_ref, rh_ref, prm_ref, gr_ref, win_ref, wsp_ref, in_sem, x_ref, go_ref,
            xt_ref, got_ref, woutt_ref, gh_ref, gl_ref, gth_ref, gtl_ref,
            fih_ref, fil_ref, fith_ref, fitl_ref, out_sem):
    srcs = (xt_hbm, got_hbm, c0, c1, c2, c3, c4, c5, c6, c7, win_hbm, wsp_hbm, woutt_hbm)
    dsts = (xt_ref, got_ref, gh_ref, gl_ref, gth_ref, gtl_ref, fih_ref, fil_ref, fith_ref, fitl_ref,
            win_ref, wsp_ref, woutt_ref)
    cps = [pltpu.make_async_copy(a_, b_, in_sem.at[i]) for i, (a_, b_) in enumerate(zip(srcs, dsts))]
    for cp in cps:
        cp.start()
    cp_o = pltpu.make_async_copy(xt_ref, ot_hbm, out_sem.at[0])
    cp_dx = pltpu.make_async_copy(got_ref, dxt_hbm, out_sem.at[1])
    cp_dwo = pltpu.make_async_copy(woutt_ref, dwoutt_hbm, out_sem.at[2])
    dt = jnp.exp(ldt_ref[...].astype(F32)).astype(BF16).astype(F32)
    dsk = dsk_ref[...].astype(F32)

    kt_ref[...] = jnp.zeros(kt_ref.shape, F32)
    for idx, r in enumerate((ar_ref, ai_ref, br_ref, bi_ref, cr_ref, ci_ref)):
        prm_ref[idx] = r[...].astype(F32).T

    def coef(n):
        row = lambda idx: prm_ref[idx, pl.ds(n, 1), :]
        zr, zi = dt * row(0), dt * row(1)
        dbr, dbi = dt * row(2), dt * row(3)
        cr, ci = _cmul(row(4), row(5), dbr, dbi)
        return zr, zi, cr, ci

    def powers(pw_ref):
        zr, zi = dt * prm_ref[0], dt * prm_ref[1]
        for j0 in (0, 5):
            pr, pi = _cexp(zr, zi, float(1 << j0))
            for j in range(j0, 5 if j0 == 0 else 11):
                pw_ref[0, j] = pr
                pw_ref[1, j] = pi
                pr, pi = pr * pr - pi * pi, 2.0 * pr * pi

    def kgen(pw_ref, n, carry):
        _, _, cr, ci = coef(n)
        coarse, fine, edge = _pre(pw_ref, n)
        for j in range(2):
            kt_ref[ESL, EACC + 8 * j:EACC + 8 * j + 8, :] += cr * edge[j][0] - ci * edge[j][1]
        for q in range(4):
            ys = [(b, t, _cmul(cr, ci, *y)) for b in range(NB) if _BLK[b][3] == q
                  for t, y in enumerate(coarse[b])]
            for r in range(_BLK[ys[0][0]][1]):
                fr = jnp.broadcast_to(fine[q][0][r:r + 1], (8, D))
                fi = jnp.broadcast_to(fine[q][1][r:r + 1], (8, D))
                for b, t, (yr, yi) in ys:
                    r0 = r * _BLK[b][2] + t * 8
                    kt_ref[b, r0:r0 + 8, :] += yr * fr - yi * fi
        return carry

    def ssm_fwd(pw_ref):
        powers(pw_ref)
        lax.fori_loop(0, N, functools.partial(kgen, pw_ref), 0)
        for b in range(2, NB):
            kt_ref[b, EDGE:EDGE + 1, :] = kt_ref[ESL, EACC + b:EACC + b + 1, :]
        kt_ref[ESL, EACC:EACC + 16, :] = jnp.zeros((16, D), F32)

    with jax.named_scope('kgen'):
        pl.run_scoped(ssm_fwd, pltpu.VMEM((2, 11, N, D), F32))

    for cp in cps[0:10]:
        cp.wait()
    for b in range(NB):
        x_ref[b * P:(b + 1) * P, :] = xt_ref[:, b * P:(b + 1) * P].astype(F32).T.astype(BF16)
        go_ref[b * P:(b + 1) * P, :] = got_ref[:, b * P:(b + 1) * P].astype(F32).T.astype(BF16)

    def spectra(uh_ref, kh_ref):
        for b in range(NB):
            u, _ = _ln(x_ref[b * P:(b + 1) * P, :].astype(F32))
            uh_ref[b] = _dot2(gh_ref[4], gl_ref[4], u)
            q = _BLK[b][3]
            kh_ref[b] = _dot3(gh_ref[q], gl_ref[q], kt_ref[b])

    def s4_fwd(uh_ref, kh_ref):
        spectra(uh_ref, kh_ref)
        prev = None
        for b in range(NB):
            zr = jnp.zeros((P, D), F32)
            zi = jnp.zeros((P, D), F32)
            for a in range(b + 1):
                pr, pi = _cmul(uh_ref[a, 0:P], uh_ref[a, P:M2], kh_ref[b - a, 0:P], kh_ref[b - a, P:M2])
                zr, zi = zr + pr, zi + pi
            zf = _dot3(fih_ref[...], fil_ref[...], jnp.concatenate([zr, zi], 0))
            y = zf[0:P] if prev is None else zf[0:P] + prev
            prev = zf[P:M2]
            xb = x_ref[b * P:(b + 1) * P, :].astype(F32)
            u, _ = _ln(xb)
            h = xb + y + u * dsk
            h_ref[b * P:(b + 1) * P, :] = h
            v, r = _ln(h)
            v_ref[b * P:(b + 1) * P, :] = v.astype(BF16)
            rh_ref[b * P:(b + 1) * P, :] = r

    with jax.named_scope('s4_fwd'):
        pl.run_scoped(s4_fwd, pltpu.VMEM((NB, M2, D), F32), pltpu.VMEM((NB, M2, D), F32))

    def gmlp(a_ref, z2_ref, r2_ref, dg_ref, acc_ref, sp_st, in_st, st_sem):
        nt = L // TR
        for cp in cps[10:13]:
            cp.wait()

        def sp_copy(i):
            return pltpu.make_async_copy(
                sp_st.at[i % 2], dwsp_hbm.at[pl.ds(pl.multiple_of(i * TR, TR), TR), :], st_sem.at[i % 2])

        def in_copy(cb):
            return pltpu.make_async_copy(
                in_st.at[cb % 2], dwin_hbm.at[:, cb * 512:(cb + 1) * 512], st_sem.at[2 + cb % 2])

        def ph_c(i, c):
            rs = pl.ds(pl.multiple_of(i * TR, TR), TR)
            a = _dot(v_ref[rs, :], win_ref[...]).astype(BF16)
            a_ref[rs, :] = a
            z2, _ = _gelu_parts(a[:, FH:].astype(F32))
            n2, r2 = _ln(z2)
            z2_ref[rs, :] = n2.astype(BF16)
            r2_ref[rs, :] = r2
            return c
        with jax.named_scope('ph_c'):
            lax.fori_loop(0, nt, ph_c, 0)

        acc_ref[...] = jnp.zeros(acc_ref.shape, F32)

        def ph_d(i, c):
            rs = pl.ds(pl.multiple_of(i * TR, TR), TR)
            g = _dot(wsp_ref[rs, :], z2_ref[...]) + bsp_ref[rs, :].astype(F32)
            z1, dg1 = _gelu_parts(a_ref[rs, 0:FH].astype(F32))
            m = (z1 * g).astype(BF16)
            xt_ref[:, rs] = (h_ref[rs, :] + _dot_nt(m, woutt_ref[...])).T.astype(BF16)
            dm = _dot(go_ref[rs, :], woutt_ref[...])
            acc_ref[...] += _dot(got_ref[:, rs], m)
            dg = dm * z1
            dbsp_ref[rs, :] = jnp.sum(dg, axis=-1, keepdims=True).astype(BF16)
            dgb = dg.astype(BF16)
            dg_ref[rs, :] = dgb

            @pl.when(i >= 2)
            def _():
                sp_copy(i - 2).wait()
            sp_st[i % 2] = _dot_nt(dgb, z2_ref[...]).astype(BF16)
            sp_copy(i).start()
            a_ref[rs, 0:FH] = (dm * g * dg1).astype(BF16)
            return c
        with jax.named_scope('ph_d'):
            lax.fori_loop(0, nt, ph_d, 0)
        woutt_ref[...] = acc_ref[...].astype(BF16)
        cp_o.start()
        cp_dwo.start()
        sp_copy(nt - 2).wait()
        sp_copy(nt - 1).wait()

        def ph_e(i, c):
            rs = pl.ds(pl.multiple_of(i * TR, TR), TR)
            dn2 = _dot_tn(wsp_ref[:, rs], dg_ref[...])
            dz2 = _ln_bwd(dn2, z2_ref[rs, :].astype(F32), r2_ref[rs, :])
            _, dg2 = _gelu_parts(a_ref[rs, FH:F].astype(F32))
            a_ref[rs, FH:F] = (dz2 * dg2).astype(BF16)
            dv = _dot_nt(a_ref[rs, :], win_ref[...])
            dh = go_ref[rs, :].astype(F32) + _ln_bwd(dv, v_ref[rs, :].astype(F32), rh_ref[rs, :])
            h_ref[rs, :] = dh
            return c
        with jax.named_scope('ph_e'):
            lax.fori_loop(0, nt, ph_e, 0)

        ncb = F // 512
        for cb in range(ncb):
            if cb >= 2:
                in_copy(cb - 2).wait()
            in_st[cb % 2] = _dot_tn(v_ref[...], a_ref[:, cb * 512:(cb + 1) * 512]).astype(BF16)
            in_copy(cb).start()
        in_copy(ncb - 2).wait()
        in_copy(ncb - 1).wait()

    pl.run_scoped(gmlp, pltpu.VMEM((L, F), BF16), pltpu.VMEM((L, FH), BF16),
                  pltpu.VMEM((L, 1), F32), pltpu.VMEM((L, FH), BF16),
                  pltpu.VMEM((D, FH), F32), pltpu.VMEM((2, TR, L), BF16),
                  pltpu.VMEM((2, D, 512), BF16), pltpu.SemaphoreType.DMA((4,)))

    def s4_bwd(uh_ref, kh_ref, dz_ref):
        spectra(uh_ref, kh_ref)
        for b in range(NB):
            dzb = _dot2(fith_ref[:, 0:P], fitl_ref[:, 0:P], h_ref[b * P:(b + 1) * P, :])
            if b + 1 < NB:
                dzb = dzb + _dot2(fith_ref[:, P:M2], fitl_ref[:, P:M2],
                                  h_ref[(b + 1) * P:(b + 2) * P, :])
            dz_ref[b] = dzb
        ddsk = jnp.zeros((1, D), F32)
        for a in range(NB):
            sr = jnp.zeros((P, D), F32)
            si = jnp.zeros((P, D), F32)
            qr = jnp.zeros((P, D), F32)
            qi = jnp.zeros((P, D), F32)
            for dlt in range(NB - a):
                zr, zi = dz_ref[a + dlt, 0:P], dz_ref[a + dlt, P:M2]
                pr, pi = _cmul(kh_ref[dlt, 0:P], -kh_ref[dlt, P:M2], zr, zi)
                sr, si = sr + pr, si + pi
                pr, pi = _cmul(uh_ref[dlt, 0:P], -uh_ref[dlt, P:M2], zr, zi)
                qr, qi = qr + pr, qi + pi
            du = _dot3(gth_ref[4], gtl_ref[4], jnp.concatenate([sr, si], 0))
            q = _BLK[a][3]
            kt_ref[a] = _dot3(gth_ref[q], gtl_ref[q], jnp.concatenate([qr, qi], 0))
            dh = h_ref[a * P:(a + 1) * P, :]
            u, r = _ln(x_ref[a * P:(a + 1) * P, :].astype(F32))
            ddsk = ddsk + jnp.sum(dh * u, axis=0, keepdims=True)
            got_ref[:, a * P:(a + 1) * P] = (dh + _ln_bwd(du + dh * dsk, u, r)).T.astype(BF16)
        ddsk_ref[...] = ddsk.astype(BF16)
        cp_dx.start()

    with jax.named_scope('s4_bwd'):
        pl.run_scoped(s4_bwd, pltpu.VMEM((NB, M2, D), F32), pltpu.VMEM((NB, M2, D), F32),
                      pltpu.VMEM((NB, M2, D), F32))

    def ssm_bwd(kv_ref, pw_ref):
        powers(pw_ref)
        kt_ref[ESL, EACC:EACC + 2, :] = jnp.zeros((2, D), F32)
        for b in range(2, NB):
            kt_ref[ESL, EACC + b:EACC + b + 1, :] = kt_ref[b, EDGE:EDGE + 1, :]
        i16 = lax.broadcasted_iota(jnp.int32, (16, 1), 0)
        kv_ref[ESL, EACC:EACC + 16, :] = kt_ref[ESL, EACC:EACC + 16, :] * ((i16 + 1) * P).astype(F32)
        for b in range(NB):
            step, nr, na, _ = _BLK[b]
            rows = nr * na
            va = (lax.broadcasted_iota(jnp.int32, (rows, 1), 0) % na) * (nr * step) + b * P
            kv_ref[b, 0:rows, :] = kt_ref[b, 0:rows, :] * va.astype(F32)

        def kbwd(n, gdt):
            _, _, cr, ci = coef(n)
            coarse, fine, edge = _pre(pw_ref, n)
            a0r = a0i = a1r = a1i = jnp.zeros((8, D), F32)
            for j in range(2):
                dk = kt_ref[ESL, EACC + 8 * j:EACC + 8 * j + 8, :]
                dv = kv_ref[ESL, EACC + 8 * j:EACC + 8 * j + 8, :]
                a0r, a0i = a0r + dk * edge[j][0], a0i + dk * edge[j][1]
                a1r, a1i = a1r + dv * edge[j][0], a1i + dv * edge[j][1]
            for q in range(4):
                ys = [(b, t, y) for b in range(NB) if _BLK[b][3] == q for t, y in enumerate(coarse[b])]
                for r in range(_BLK[ys[0][0]][1]):
                    w0r = w0i = w1r = w1i = None
                    for b, t, (yr, yi) in ys:
                        r0 = r * _BLK[b][2] + t * 8
                        dk, dv = kt_ref[b, r0:r0 + 8, :], kv_ref[b, r0:r0 + 8, :]
                        if w0r is None:
                            w0r, w0i, w1r, w1i = dk * yr, dk * yi, dv * yr, dv * yi
                        else:
                            w0r, w0i = w0r + dk * yr, w0i + dk * yi
                            w1r, w1i = w1r + dv * yr, w1i + dv * yi
                    vb = float(r << q)
                    w1r, w1i = w1r + vb * w0r, w1i + vb * w0i
                    fr = jnp.broadcast_to(fine[q][0][r:r + 1], (8, D))
                    fi = jnp.broadcast_to(fine[q][1][r:r + 1], (8, D))
                    pr, pi = _cmul(w0r, w0i, fr, fi)
                    a0r, a0i = a0r + pr, a0i + pi
                    pr, pi = _cmul(w1r, w1i, fr, fi)
                    a1r, a1i = a1r + pr, a1i + pi
            red = lambda t: jnp.sum(t, axis=0, keepdims=True)
            s0r, s0i, s1r, s1i = red(a0r), red(a0i), red(a1r), red(a1i)
            gcr, gci = s0r, -s0i
            wr, wi = _cmul(cr, ci, s1r, s1i)
            gzr, gzi = wr, -wi
            row = lambda idx: prm_ref[idx, pl.ds(n, 1), :]
            cre, cim, bre, bim = row(4), row(5), row(2), row(3)
            dbr, dbi = dt * bre, dt * bim
            gdbr = gcr * cre + gci * cim
            gdbi = gci * cre - gcr * cim
            gr_ref[4, pl.ds(n, 1), :] = gcr * dbr + gci * dbi
            gr_ref[5, pl.ds(n, 1), :] = gci * dbr - gcr * dbi
            gr_ref[2, pl.ds(n, 1), :] = dt * gdbr
            gr_ref[3, pl.ds(n, 1), :] = dt * gdbi
            gr_ref[0, pl.ds(n, 1), :] = dt * gzr
            gr_ref[1, pl.ds(n, 1), :] = dt * gzi
            return gdt + gdbr * bre + gdbi * bim + gzr * row(0) + gzi * row(1)
        with jax.named_scope('kbwd'):
            gdt = lax.fori_loop(0, N, kbwd, jnp.zeros((1, D), F32))
        dldt_ref[...] = (gdt * dt).astype(BF16)

    pl.run_scoped(ssm_bwd, pltpu.VMEM((NB, P, D), F32), pltpu.VMEM((2, 11, N, D), F32))
    for idx, r in enumerate((dar_ref, dai_ref, dbr_ref, dbi_ref, dcr_ref, dci_ref)):
        r[...] = gr_ref[idx].T.astype(BF16)
    cp_o.wait()
    cp_dwo.wait()
    cp_dx.wait()


@jax.jit
def pallas_sequential_preLN__ssm_conv_s4__mixer_gmlp__prompt_kernel(
    A_u, A_A_re, A_A_im, A_B_re, A_B_im, A_C_re, A_C_im, A_log_dt, A_Dskip,
    B_x, B_w_in, B_w_sp, B_b_sp, B_w_out, grad_out,
):
    del B_x
    consts = _consts()
    sds = jax.ShapeDtypeStruct
    out_shape = (
        sds((D, L), BF16), sds((D, L), BF16),
        sds((D, N), BF16), sds((D, N), BF16), sds((D, N), BF16),
        sds((D, N), BF16), sds((D, N), BF16), sds((D, N), BF16),
        sds((1, D), BF16), sds((1, D), BF16),
        sds((D, F), BF16), sds((L, L), BF16), sds((L, 1), BF16), sds((D, FH), BF16),
    )
    vm = pl.BlockSpec(memory_space=pltpu.VMEM)
    hbm = pl.BlockSpec(memory_space=pl.ANY)
    outs = pl.pallas_call(
        _kernel,
        out_shape=out_shape,
        in_specs=[hbm if (i in (0, 9, 10, 12, 13) or i >= 14) else vm for i in range(14 + len(consts))],
        out_specs=tuple(hbm if i in (0, 1, 10, 11, 13) else vm for i in range(14)),
        scratch_shapes=[
            pltpu.VMEM((NB, P, D), F32),
            pltpu.VMEM((L, D), BF16),
            pltpu.VMEM((L, D), F32),
            pltpu.VMEM((L, 1), F32),
            pltpu.VMEM((6, N, D), F32),
            pltpu.VMEM((6, N, D), F32),
            pltpu.VMEM((D, F), BF16),
            pltpu.VMEM((L, L), BF16),
            pltpu.SemaphoreType.DMA((13,)),
            pltpu.VMEM((L, D), BF16),
            pltpu.VMEM((L, D), BF16),
            pltpu.VMEM((D, L), BF16),
            pltpu.VMEM((D, L), BF16),
            pltpu.VMEM((D, FH), BF16),
            *[pltpu.VMEM(c.shape, BF16) for c in consts],
            pltpu.SemaphoreType.DMA((3,)),
        ],
        compiler_params=pltpu.CompilerParams(vmem_limit_bytes=120 * 1024 * 1024),
    )(A_u.reshape(L, D).T, A_A_re, A_A_im, A_B_re, A_B_im, A_C_re, A_C_im,
      A_log_dt.reshape(1, D), A_Dskip.reshape(1, D), B_w_in, B_w_sp,
      B_b_sp.reshape(L, 1), B_w_out.T, grad_out.reshape(L, D).T, *consts)
    (o, dx, dar, dai, dbr, dbi, dcr, dci, dldt, ddsk, dwin, dwsp, dbsp, dwout) = outs
    return (o.T.reshape(1, L, D), dx.T.reshape(1, L, D), dar, dai, dbr, dbi, dcr, dci,
            dldt.reshape(D), ddsk.reshape(D), dwin, dwsp, dbsp.reshape(L), dwout.T)
```

```python
import functools
import numpy as np
import ml_dtypes
import jax
import jax.numpy as jnp
from jax import lax
import jax.experimental.pallas as pl
import jax.experimental.pallas.tpu as pltpu

L = 2048
D = 576
N = 128
FH = 2304
F = 2 * FH
P = 128
NB = L // P
M2 = 2 * P
EPS = 1e-5
TR = 256
F32 = jnp.float32
BF16 = jnp.bfloat16

_BLK = [(1, 8, 16, 0)] * 2 + [(2, 8, 8, 1)] * 2 + [(4, 4, 8, 2)] * 4 + [(8, 2, 8, 3)] * 8
EDGE = 120
EACC = 96
ESL = 2


def _split(a):
    a = np.asarray(a, np.float64)
    hi = a.astype(np.float32).astype(ml_dtypes.bfloat16)
    lo = (a - hi.astype(np.float64)).astype(np.float32).astype(ml_dtypes.bfloat16)
    return hi, lo


def _consts():
    k = np.arange(P)
    om = np.pi * (2 * k + 1) / M2
    j = np.arange(P)
    fw = np.concatenate([np.cos(np.outer(om, j)), -np.sin(np.outer(om, j))], 0)
    t = np.arange(M2)
    fi = np.concatenate([np.cos(np.outer(t, om)), -np.sin(np.outer(t, om))], 1) * (2.0 / M2)
    lb = np.arange(L).astype(np.float32).astype(ml_dtypes.bfloat16).astype(np.float64).astype(np.int64)
    gs = []
    for blk in (0, 2, 4, 8):
        step, nr, na, _ = _BLK[blk]
        g = np.zeros((M2, P))
        for jj in range(P):
            m = (lb[blk * P + jj] - blk * P) // step
            col = EDGE if m == nr * na else (m % nr) * na + m // nr
            g[:, col] += fw[:, jj]
        gs.append(g)
    gs.append(fw)
    gs = np.stack(gs)
    gts = np.transpose(gs, (0, 2, 1))
    out = []
    for a in (gs, gts, fi, fi.T):
        out.extend(_split(a))
    return out


def _dot(a, b):
    return jnp.dot(a, b, preferred_element_type=F32)


def _dot_nt(a, b):
    return lax.dot_general(a, b, (((1,), (1,)), ((), ())), preferred_element_type=F32)


def _dot_tn(a, b):
    return lax.dot_general(a, b, (((0,), (0,)), ((), ())), preferred_element_type=F32)


def _dot3(mh, ml, x):
    xh = x.astype(BF16)
    xl = (x - xh.astype(F32)).astype(BF16)
    return _dot(mh, xh) + (_dot(mh, xl) + _dot(ml, xh))


def _dot2(mh, ml, x):
    xh = x.astype(BF16)
    return _dot(mh, xh) + _dot(ml, xh)


def _ln(x):
    mu = jnp.mean(x, axis=-1, keepdims=True)
    xc = x - mu
    var = jnp.mean(xc * xc, axis=-1, keepdims=True)
    r = lax.rsqrt(var + EPS)
    return xc * r, r


def _ln_bwd(dn, n, r):
    return r * (dn - jnp.mean(dn, axis=-1, keepdims=True)
                - n * jnp.mean(dn * n, axis=-1, keepdims=True))


_GK = 0.7978845608028654
_GC = 0.044715


def _gelu_parts(a):
    t = jnp.tanh(_GK * (a + _GC * a * a * a))
    g = 0.5 * a * (1.0 + t)
    dg = 0.5 * (1.0 + t) + 0.5 * a * (1.0 - t * t) * _GK * (1.0 + 3.0 * _GC * a * a)
    return g, dg


def _cmul(ar, ai, br, bi):
    return ar * br - ai * bi, ar * bi + ai * br


def _cexp(zr, zi, mult):
    e = jnp.exp(zr * mult)
    ang = zi * mult
    return e * jnp.cos(ang), e * jnp.sin(ang)


def _pre(pw_ref, n):
    rows = [(pw_ref[0, j, pl.ds(n, 1), :], pw_ref[1, j, pl.ds(n, 1), :]) for j in range(11)]
    e = lambda j: rows[j]
    i8 = lax.broadcasted_iota(jnp.int32, (8, 1), 0)

    def tile3(q):
        fs = []
        for bit in range(3):
            on = ((i8 >> bit) & 1) == 1
            fs.append((jnp.where(on, rows[q + bit][0], 1.0), jnp.where(on, rows[q + bit][1], 0.0)))
        return _cmul(*_cmul(*fs[0], *fs[1]), *fs[2])

    fine = [tile3(q) for q in range(4)]
    t3, t4 = tile3(3), tile3(4)
    olo = tile3(7)
    ohi = _cmul(*olo, *e(10))
    off = lambda b: tuple(x[b % 8:b % 8 + 1] for x in (olo if b < 8 else ohi))
    t36 = _cmul(*t3, *e(6))
    coarse = [[t3, t36], [_cmul(*t3, *e(7)), _cmul(*t36, *e(7))]]
    coarse += [[_cmul(*t4, *off(b))] for b in range(2, NB)]
    edge = [_cmul(*olo, *e(7)), _cmul(*ohi, *e(7))]
    return coarse, fine, edge


def _kernel(xt_hbm, ar_ref, ai_ref, br_ref, bi_ref, cr_ref, ci_ref, ldt_ref, dsk_ref,
            win_hbm, wsp_hbm, bsp_ref, woutt_hbm, got_hbm,
            c0, c1, c2, c3, c4, c5, c6, c7,
            ot_hbm, dxt_hbm, dar_ref, dai_ref, dbr_ref, dbi_ref, dcr_ref, dci_ref,
            dldt_ref, ddsk_ref, dwin_hbm, dwsp_hbm, dbsp_ref, dwoutt_hbm,
            kt_ref, v_ref, h_ref, rh_ref, prm_ref, in_sem, x_ref,
            xt_ref, got_ref, woutt_ref, gh_ref, gl_ref, gth_ref, gtl_ref,
            fih_ref, fil_ref, fith_ref, fitl_ref, out_sem,
            a_ref, z2_ref, dg_ref, sp_st, in_st, st_sem):
    srcs = (xt_hbm, got_hbm, c0, c1, c2, c3, c4, c5, c6, c7, woutt_hbm)
    dsts = (xt_ref, got_ref, gh_ref, gl_ref, gth_ref, gtl_ref, fih_ref, fil_ref, fith_ref, fitl_ref, woutt_ref)
    cps = [pltpu.make_async_copy(a_, b_, in_sem.at[i]) for i, (a_, b_) in enumerate(zip(srcs, dsts))]
    for cp in cps:
        cp.start()
    cp_o = pltpu.make_async_copy(xt_ref, ot_hbm, out_sem.at[0])
    cp_dx = pltpu.make_async_copy(got_ref, dxt_hbm, out_sem.at[1])
    cp_dwo = pltpu.make_async_copy(woutt_ref, dwoutt_hbm, out_sem.at[2])
    dt = jnp.exp(ldt_ref[...].astype(F32)).astype(BF16).astype(F32)
    dsk = dsk_ref[...].astype(F32)

    kt_ref[...] = jnp.zeros(kt_ref.shape, F32)
    for idx, r in enumerate((ar_ref, ai_ref, br_ref, bi_ref, cr_ref, ci_ref)):
        prm_ref[idx] = r[...].astype(F32).T

    def coef(n):
        row = lambda idx: prm_ref[idx, pl.ds(n, 1), :]
        zr, zi = dt * row(0), dt * row(1)
        dbr, dbi = dt * row(2), dt * row(3)
        cr, ci = _cmul(row(4), row(5), dbr, dbi)
        return zr, zi, cr, ci

    def powers(pw_ref):
        zr, zi = dt * prm_ref[0], dt * prm_ref[1]
        for j0 in (0, 5):
            pr, pi = _cexp(zr, zi, float(1 << j0))
            for j in range(j0, 5 if j0 == 0 else 11):
                pw_ref[0, j] = pr
                pw_ref[1, j] = pi
                pr, pi = pr * pr - pi * pi, 2.0 * pr * pi

    def kgen(pw_ref, n, carry):
        _, _, cr, ci = coef(n)
        coarse, fine, edge = _pre(pw_ref, n)
        for j in range(2):
            kt_ref[ESL, EACC + 8 * j:EACC + 8 * j + 8, :] += cr * edge[j][0] - ci * edge[j][1]
        for q in range(4):
            ys = [(b, t, _cmul(cr, ci, *y)) for b in range(NB) if _BLK[b][3] == q
                  for t, y in enumerate(coarse[b])]
            for r in range(_BLK[ys[0][0]][1]):
                fr = jnp.broadcast_to(fine[q][0][r:r + 1], (8, D))
                fi = jnp.broadcast_to(fine[q][1][r:r + 1], (8, D))
                for b, t, (yr, yi) in ys:
                    r0 = r * _BLK[b][2] + t * 8
                    kt_ref[b, r0:r0 + 8, :] += yr * fr - yi * fi
        return carry

    def ssm_fwd(pw_ref):
        powers(pw_ref)
        lax.fori_loop(0, N, functools.partial(kgen, pw_ref), 0)
        for b in range(2, NB):
            kt_ref[b, EDGE:EDGE + 1, :] = kt_ref[ESL, EACC + b:EACC + b + 1, :]
        kt_ref[ESL, EACC:EACC + 16, :] = jnp.zeros((16, D), F32)

    def spectra(uh_ref, kh_ref):
        for b in range(NB):
            u, _ = _ln(x_ref[b * P:(b + 1) * P, :].astype(F32))
            uh_ref[b] = _dot2(gh_ref[4], gl_ref[4], u)
            q = _BLK[b][3]
            kh_ref[b] = _dot3(gh_ref[q], gl_ref[q], kt_ref[b])

    def s4_fwd(uh_ref, kh_ref):
        spectra(uh_ref, kh_ref)
        prev = None
        for b in range(NB):
            zr = jnp.zeros((P, D), F32)
            zi = jnp.zeros((P, D), F32)
            for a in range(b + 1):
                pr, pi = _cmul(uh_ref[a, 0:P], uh_ref[a, P:M2], kh_ref[b - a, 0:P], kh_ref[b - a, P:M2])
                zr, zi = zr + pr, zi + pi
            zf = _dot3(fih_ref[...], fil_ref[...], jnp.concatenate([zr, zi], 0))
            y = zf[0:P] if prev is None else zf[0:P] + prev
            prev = zf[P:M2]
            xb = x_ref[b * P:(b + 1) * P, :].astype(F32)
            u, _ = _ln(xb)
            h = xb + y + u * dsk
            h_ref[b * P:(b + 1) * P, :] = h
            v, r = _ln(h)
            v_ref[b * P:(b + 1) * P, :] = v.astype(BF16)
            rh_ref[b * P:(b + 1) * P, 0:1] = r

    def back():
        def gmlp(win_ref, wsp_ref, acc_ref):
            nt = L // TR


            def ph_c(i, c):
                rs = pl.ds(pl.multiple_of(i * TR, TR), TR)
                a = _dot(v_ref[rs, :], win_ref[...]).astype(BF16)
                a_ref[rs, :] = a
                z2, _ = _gelu_parts(a[:, FH:].astype(F32))
                n2, r2 = _ln(z2)
                z2_ref[rs, :] = n2.astype(BF16)
                rh_ref[rs, 1:2] = r2
                return c
            with jax.named_scope('ph_c'):
                lax.fori_loop(0, nt, ph_c, 0)

            acc_ref[...] = jnp.zeros(acc_ref.shape, F32)

            def ph_d(i, c):
                rs = pl.ds(pl.multiple_of(i * TR, TR), TR)
                o = h_ref[rs, :]
                dbs = jnp.zeros((TR, 1), F32)
                go = got_ref[:, rs].astype(F32).T.astype(BF16)
                hw = FH // 2
                for c0 in (0, hw):
                    cs = slice(c0, c0 + hw)
                    g = _dot(wsp_ref[rs, :], z2_ref[:, cs]) + bsp_ref[rs, :].astype(F32)
                    z1, dg1 = _gelu_parts(a_ref[rs, cs].astype(F32))
                    m = (z1 * g).astype(BF16)
                    o = o + _dot_nt(m, woutt_ref[:, cs])
                    dm = _dot(go, woutt_ref[:, cs])
                    acc_ref[:, cs] += _dot(got_ref[:, rs], m)
                    dg = dm * z1
                    dbs = dbs + jnp.sum(dg, axis=-1, keepdims=True)
                    dg_ref[rs, cs] = dg.astype(BF16)
                    a_ref[rs, cs] = (dm * g * dg1).astype(BF16)
                xt_ref[:, rs] = o.T.astype(BF16)
                dbsp_ref[rs, :] = dbs.astype(BF16)
                return c
            with jax.named_scope('ph_d'):
                lax.fori_loop(0, nt, ph_d, 0)
            woutt_ref[...] = acc_ref[...].astype(BF16)
            cp_o.start()
            cp_dwo.start()

            def ph_e(i, c):
                rs = pl.ds(pl.multiple_of(i * TR, TR), TR)
                dn2 = _dot_tn(wsp_ref[:, rs], dg_ref[...])
                dz2 = _ln_bwd(dn2, z2_ref[rs, :].astype(F32), rh_ref[rs, 1:2])
                _, dg2 = _gelu_parts(a_ref[rs, FH:F].astype(F32))
                a_ref[rs, FH:F] = (dz2 * dg2).astype(BF16)
                dv = _dot_nt(a_ref[rs, :], win_ref[...])
                dh = got_ref[:, rs].astype(F32).T + _ln_bwd(dv, v_ref[rs, :].astype(F32), rh_ref[rs, 0:1])
                h_ref[rs, :] = dh
                return c
            with jax.named_scope('ph_e'):
                lax.fori_loop(0, nt, ph_e, 0)

        def front(win_ref, wsp_ref):
            wcps = [pltpu.make_async_copy(win_hbm, win_ref, in_sem.at[11]),
                    pltpu.make_async_copy(wsp_hbm, wsp_ref, in_sem.at[12])]
            for cp in wcps:
                cp.start()
            with jax.named_scope('kgen'):
                pl.run_scoped(ssm_fwd, pltpu.VMEM((2, 11, N, D), F32))

            for cp in cps[0:10]:
                cp.wait()
            for b in range(NB):
                x_ref[b * P:(b + 1) * P, :] = xt_ref[:, b * P:(b + 1) * P].astype(F32).T.astype(BF16)

            with jax.named_scope('s4_fwd'):
                pl.run_scoped(s4_fwd, pltpu.VMEM((NB, M2, D), F32), pltpu.VMEM((NB, M2, D), F32))

            for cp in [cps[10]] + wcps:
                cp.wait()
            pl.run_scoped(functools.partial(gmlp, win_ref, wsp_ref),
                          pltpu.VMEM((D, FH), F32))

        pl.run_scoped(front, pltpu.VMEM((D, F), BF16), pltpu.VMEM((L, L), BF16))

        def s4_bwd(uh_ref, kh_ref, dz_ref):
            spectra(uh_ref, kh_ref)
            for b in range(NB):
                dzb = _dot2(fith_ref[:, 0:P], fitl_ref[:, 0:P], h_ref[b * P:(b + 1) * P, :])
                if b + 1 < NB:
                    dzb = dzb + _dot2(fith_ref[:, P:M2], fitl_ref[:, P:M2],
                                      h_ref[(b + 1) * P:(b + 2) * P, :])
                dz_ref[b] = dzb
            ddsk = jnp.zeros((1, D), F32)
            for a in range(NB):
                sr = jnp.zeros((P, D), F32)
                si = jnp.zeros((P, D), F32)
                qr = jnp.zeros((P, D), F32)
                qi = jnp.zeros((P, D), F32)
                for dlt in range(NB - a):
                    zr, zi = dz_ref[a + dlt, 0:P], dz_ref[a + dlt, P:M2]
                    pr, pi = _cmul(kh_ref[dlt, 0:P], -kh_ref[dlt, P:M2], zr, zi)
                    sr, si = sr + pr, si + pi
                    pr, pi = _cmul(uh_ref[dlt, 0:P], -uh_ref[dlt, P:M2], zr, zi)
                    qr, qi = qr + pr, qi + pi
                du = _dot3(gth_ref[4], gtl_ref[4], jnp.concatenate([sr, si], 0))
                q = _BLK[a][3]
                kt_ref[a] = _dot3(gth_ref[q], gtl_ref[q], jnp.concatenate([qr, qi], 0))
                dh = h_ref[a * P:(a + 1) * P, :]
                u, r = _ln(x_ref[a * P:(a + 1) * P, :].astype(F32))
                ddsk = ddsk + jnp.sum(dh * u, axis=0, keepdims=True)
                got_ref[:, a * P:(a + 1) * P] = (dh + _ln_bwd(du + dh * dsk, u, r)).T.astype(BF16)
            ddsk_ref[...] = ddsk.astype(BF16)
            cp_dx.start()

        with jax.named_scope('s4_bwd'):
            pl.run_scoped(s4_bwd, pltpu.VMEM((NB, M2, D), F32), pltpu.VMEM((NB, M2, D), F32),
                          pltpu.VMEM((NB, M2, D), F32))

        def ssm_bwd(kv_ref, pw_ref, vt_ref, gr_ref):
            for b in range(NB):
                vt_ref[:, b * P:(b + 1) * P] = v_ref[b * P:(b + 1) * P, :].astype(F32).T.astype(BF16)
            powers(pw_ref)
            kt_ref[ESL, EACC:EACC + 2, :] = jnp.zeros((2, D), F32)
            for b in range(2, NB):
                kt_ref[ESL, EACC + b:EACC + b + 1, :] = kt_ref[b, EDGE:EDGE + 1, :]
            i16 = lax.broadcasted_iota(jnp.int32, (16, 1), 0)
            kv_ref[ESL, EACC:EACC + 16, :] = kt_ref[ESL, EACC:EACC + 16, :] * ((i16 + 1) * P).astype(F32)
            for b in range(NB):
                step, nr, na, _ = _BLK[b]
                rows = nr * na
                va = (lax.broadcasted_iota(jnp.int32, (rows, 1), 0) % na) * (nr * step) + b * P
                kv_ref[b, 0:rows, :] = kt_ref[b, 0:rows, :] * va.astype(F32)

            def sp_copy(n):
                return pltpu.make_async_copy(
                    sp_st.at[n % 2],
                    dwsp_hbm.at[pl.ds(pl.multiple_of((n // 16) * 256, 256), 256),
                                pl.ds(pl.multiple_of((n % 16) * 128, 128), 128)], st_sem.at[n % 2])

            def in_copy(n):
                return pltpu.make_async_copy(
                    in_st.at[n % 2],
                    dwin_hbm.at[pl.ds(pl.multiple_of((n // 36) * 144, 16), 144),
                                pl.ds(pl.multiple_of((n % 36) * 128, 128), 128)], st_sem.at[2 + n % 2])

            def in_tile(n):
                in_st[n % 2] = _dot(
                    vt_ref[pl.ds(pl.multiple_of((n // 36) * 144, 16), 144), :],
                    a_ref[:, pl.ds(pl.multiple_of((n % 36) * 128, 128), 128)]).astype(BF16)

            for n in range(N, 144):
                if n >= N + 2:
                    in_copy(n - 2).wait()
                in_tile(n)
                in_copy(n).start()
            in_copy(142).wait()
            in_copy(143).wait()

            def kbwd(n, gdt):
                @pl.when(n >= 2)
                def _():
                    sp_copy(n - 2).wait()
                    in_copy(n - 2).wait()
                t_rows = pl.ds(pl.multiple_of((n // 16) * 256, 256), 256)
                s_rows = pl.ds(pl.multiple_of((n % 16) * 128, 128), 128)
                d_rows = pl.ds(pl.multiple_of((n // 36) * 144, 16), 144)
                f_cols = pl.ds(pl.multiple_of((n % 36) * 128, 128), 128)
                jobs = [("s", k) for k in range(FH // 128)] + [("i", k) for k in range(L // 128)]
                accs = {"s": None, "i": None}

                def run_jobs(cnt):
                    for _ in range(cnt):
                        if not jobs:
                            return
                        kind, k = jobs.pop(0)
                        ks = slice(k * 128, (k + 1) * 128)
                        if kind == "s":
                            d = _dot_nt(dg_ref[t_rows, ks], z2_ref[s_rows, ks])
                        else:
                            d = _dot(vt_ref[d_rows, ks], a_ref[ks, f_cols])
                        accs[kind] = d if accs[kind] is None else accs[kind] + d

                _, _, cr, ci = coef(n)
                coarse, fine, edge = _pre(pw_ref, n)
                a0r = a0i = a1r = a1i = jnp.zeros((8, D), F32)
                for j in range(2):
                    dk = kt_ref[ESL, EACC + 8 * j:EACC + 8 * j + 8, :]
                    dv = kv_ref[ESL, EACC + 8 * j:EACC + 8 * j + 8, :]
                    a0r, a0i = a0r + dk * edge[j][0], a0i + dk * edge[j][1]
                    a1r, a1i = a1r + dv * edge[j][0], a1i + dv * edge[j][1]
                for q in range(4):
                    ys = [(b, t, y) for b in range(NB) if _BLK[b][3] == q for t, y in enumerate(coarse[b])]
                    for r in range(_BLK[ys[0][0]][1]):
                        w0r = w0i = w1r = w1i = None
                        run_jobs(2 if q < 2 else 1)
                        for b, t, (yr, yi) in ys:
                            r0 = r * _BLK[b][2] + t * 8
                            dk, dv = kt_ref[b, r0:r0 + 8, :], kv_ref[b, r0:r0 + 8, :]
                            if w0r is None:
                                w0r, w0i, w1r, w1i = dk * yr, dk * yi, dv * yr, dv * yi
                            else:
                                w0r, w0i = w0r + dk * yr, w0i + dk * yi
                                w1r, w1i = w1r + dv * yr, w1i + dv * yi
                        vb = float(r << q)
                        w1r, w1i = w1r + vb * w0r, w1i + vb * w0i
                        fr = jnp.broadcast_to(fine[q][0][r:r + 1], (8, D))
                        fi = jnp.broadcast_to(fine[q][1][r:r + 1], (8, D))
                        pr, pi = _cmul(w0r, w0i, fr, fi)
                        a0r, a0i = a0r + pr, a0i + pi
                        pr, pi = _cmul(w1r, w1i, fr, fi)
                        a1r, a1i = a1r + pr, a1i + pi
                run_jobs(100)
                sp_st[n % 2] = accs["s"].astype(BF16)
                in_st[n % 2] = accs["i"].astype(BF16)
                sp_copy(n).start()
                in_copy(n).start()
                red = lambda t: jnp.sum(t, axis=0, keepdims=True)
                s0r, s0i, s1r, s1i = red(a0r), red(a0i), red(a1r), red(a1i)
                gcr, gci = s0r, -s0i
                wr, wi = _cmul(cr, ci, s1r, s1i)
                gzr, gzi = wr, -wi
                row = lambda idx: prm_ref[idx, pl.ds(n, 1), :]
                cre, cim, bre, bim = row(4), row(5), row(2), row(3)
                dbr, dbi = dt * bre, dt * bim
                gdbr = gcr * cre + gci * cim
                gdbi = gci * cre - gcr * cim
                gr_ref[4, pl.ds(n, 1), :] = gcr * dbr + gci * dbi
                gr_ref[5, pl.ds(n, 1), :] = gci * dbr - gcr * dbi
                gr_ref[2, pl.ds(n, 1), :] = dt * gdbr
                gr_ref[3, pl.ds(n, 1), :] = dt * gdbi
                gr_ref[0, pl.ds(n, 1), :] = dt * gzr
                gr_ref[1, pl.ds(n, 1), :] = dt * gzi
                return gdt + gdbr * bre + gdbi * bim + gzr * row(0) + gzi * row(1)
            with jax.named_scope('kbwd'):
                gdt = lax.fori_loop(0, N, kbwd, jnp.zeros((1, D), F32))
            dldt_ref[...] = (gdt * dt).astype(BF16)
            for idx, r in enumerate((dar_ref, dai_ref, dbr_ref, dbi_ref, dcr_ref, dci_ref)):
                r[...] = gr_ref[idx].T.astype(BF16)
            for n in (N - 2, N - 1):
                sp_copy(n).wait()
                in_copy(n).wait()

        pl.run_scoped(ssm_bwd, pltpu.VMEM((NB, P, D), F32), pltpu.VMEM((2, 11, N, D), F32),
                      pltpu.VMEM((D, L), BF16), pltpu.VMEM((6, N, D), F32))
    back()
    cp_o.wait()
    cp_dwo.wait()
    cp_dx.wait()


@jax.jit
def pallas_sequential_preLN__ssm_conv_s4__mixer_gmlp__prompt_kernel(
    A_u, A_A_re, A_A_im, A_B_re, A_B_im, A_C_re, A_C_im, A_log_dt, A_Dskip,
    B_x, B_w_in, B_w_sp, B_b_sp, B_w_out, grad_out,
):
    del B_x
    consts = _consts()
    sds = jax.ShapeDtypeStruct
    out_shape = (
        sds((D, L), BF16), sds((D, L), BF16),
        sds((D, N), BF16), sds((D, N), BF16), sds((D, N), BF16),
        sds((D, N), BF16), sds((D, N), BF16), sds((D, N), BF16),
        sds((1, D), BF16), sds((1, D), BF16),
        sds((D, F), BF16), sds((L, L), BF16), sds((L, 1), BF16), sds((D, FH), BF16),
    )
    vm = pl.BlockSpec(memory_space=pltpu.VMEM)
    hbm = pl.BlockSpec(memory_space=pl.ANY)
    outs = pl.pallas_call(
        _kernel,
        out_shape=out_shape,
        in_specs=[hbm if (i in (0, 9, 10, 12, 13) or i >= 14) else vm for i in range(14 + len(consts))],
        out_specs=tuple(hbm if i in (0, 1, 10, 11, 13) else vm for i in range(14)),
        scratch_shapes=[
            pltpu.VMEM((NB, P, D), F32),
            pltpu.VMEM((L, D), BF16),
            pltpu.VMEM((L, D), F32),
            pltpu.VMEM((L, 2), F32),
            pltpu.VMEM((6, N, D), F32),
            pltpu.SemaphoreType.DMA((13,)),
            pltpu.VMEM((L, D), BF16),
            pltpu.VMEM((D, L), BF16),
            pltpu.VMEM((D, L), BF16),
            pltpu.VMEM((D, FH), BF16),
            *[pltpu.VMEM(c.shape, BF16) for c in consts],
            pltpu.SemaphoreType.DMA((3,)),
            pltpu.VMEM((L, F), BF16),
            pltpu.VMEM((L, FH), BF16),
            pltpu.VMEM((L, FH), BF16),
            pltpu.VMEM((2, 256, 128), BF16), pltpu.VMEM((2, 144, 128), BF16),
            pltpu.SemaphoreType.DMA((4,)),
        ],
        compiler_params=pltpu.CompilerParams(vmem_limit_bytes=126 * 1024 * 1024),
    )(A_u.reshape(L, D).T, A_A_re, A_A_im, A_B_re, A_B_im, A_C_re, A_C_im,
      A_log_dt.reshape(1, D), A_Dskip.reshape(1, D), B_w_in, B_w_sp,
      B_b_sp.reshape(L, 1), B_w_out.T, grad_out.reshape(L, D).T, *consts)
    (o, dx, dar, dai, dbr, dbi, dcr, dci, dldt, ddsk, dwin, dwsp, dbsp, dwout) = outs
    return (o.T.reshape(1, L, D), dx.T.reshape(1, L, D), dar, dai, dbr, dbi, dcr, dci,
            dldt.reshape(D), ddsk.reshape(D), dwin, dwsp, dbsp.reshape(L), dwout.T)
```
